```python
import os as _os
_os.environ.setdefault("JAX_PLATFORMS", "cpu")
import jax
import jax.numpy as jnp

def _softmax(x, axis=-1):
    return jax.nn.softmax(x, axis=axis)
def _gelu(x):
    return jax.nn.gelu(x, approximate=True)
def _silu(x):
    return jax.nn.silu(x)
def _sigmoid(x):
    return jax.nn.sigmoid(x)
def _layernorm(x, axis=-1, eps=1e-5):
    m = jnp.mean(x, axis=axis, keepdims=True)
    v = jnp.var(x, axis=axis, keepdims=True)
    return (x - m) / jnp.sqrt(v + eps)
def _scatter_add(tgt, idx, src, axis=0):
    return tgt.at[idx].add(src)
def _segment_sum(src, seg, n):
    return jax.ops.segment_sum(src, seg, n)
class _Rng:
    def __init__(self, key):
        self._k = key
    def _next(self):
        self._k, sub = jax.random.split(self._k)
        return sub
    def normal(self, shape):
        return jax.random.normal(self._next(), shape, dtype=jnp.bfloat16)
    def randint(self, lo, hi, shape):
        return jax.random.randint(self._next(), shape, lo, hi, dtype=jnp.int32)
    def uniform(self, shape, lo=0.0, hi=1.0):
        return jax.random.uniform(self._next(), shape, jnp.bfloat16, lo, hi)
    def permutation(self, n):
        return jax.random.permutation(self._next(), n)


kernel_name = 'sequential_preLN__softmax_full_mha__swiglu_ffn__prompt'

def setup_inputs():
    _rng = _Rng(jax.random.key(int.from_bytes(__import__("os").urandom(4), "little")))
    _w = (lambda a: (lambda t: t.astype(jnp.bfloat16) if jnp.issubdtype(t.dtype, jnp.floating) else t)(jnp.asarray(a)))
    def _A_setup():
        B, S, D = 1, 2048, 512
        return {
            "x": _w((lambda *s: _rng.normal(s) * 0.05)(B, S, D)),
            "wqkv": _w((lambda *s: _rng.normal(s) * 0.05)(D, 3 * D)),
            "wo": _w((lambda *s: _rng.normal(s) * 0.05)(D, D)),
        }
    _A_in = _A_setup()

    def _B_setup():
        B, S, D, F = 1, 2048, 512, 1792
        return {
            "x": _w((lambda *s: _rng.normal(s) * 0.05)(B, S, D)),
            "w_gate": _w((lambda *s: _rng.normal(s) * 0.05)(D, F)),
            "w_up": _w((lambda *s: _rng.normal(s) * 0.05)(D, F)),
            "w_down": _w((lambda *s: _rng.normal(s) * 0.05)(F, D)),
        }
    _B_in = _B_setup()

    return {
        "A_x": _A_in["x"],
        "A_wqkv": _A_in["wqkv"],
        "A_wo": _A_in["wo"],
        "B_x": _B_in["x"],
        "B_w_gate": _B_in["w_gate"],
        "B_w_up": _B_in["w_up"],
        "B_w_down": _B_in["w_down"],
    }

def reference(A_x, A_wqkv, A_wo, B_x, B_w_gate, B_w_up, B_w_down):
    def _A_ref(x, wqkv, wo):
        B, S, D = x.shape
        H = 32; Dh = D // H
        qkv = (lambda x, *d: x.transpose(*d))((x @ wqkv).reshape(B, S, 3, H, Dh), 2, 0, 3, 1, 4)
        q, k, v = qkv[0], qkv[1], qkv[2]
        scale = Dh ** -0.5
        scores = jnp.einsum("bhqd,bhkd->bhqk", q, k) * scale
        p = _softmax(scores, axis=-1)
        o = jnp.einsum("bhqk,bhkd->bhqd", p, v)
        return (lambda x, *d: x.transpose(*d))(o, 0, 2, 1, 3).reshape(B, S, D) @ wo

    def _B_ref(x, w_gate, w_up, w_down):
        g = _silu(x @ w_gate)
        u = x @ w_up
        return (g * u) @ w_down

    x = A_x
    h = x + _A_ref(_layernorm(x, axis=-1), A_wqkv, A_wo)
    h2 = h + _B_ref(_layernorm(h, axis=-1), B_w_gate, B_w_up, B_w_down)
    return h2
```

```python
import functools
import math

import jax
import jax.numpy as jnp
from jax import lax
import jax.experimental.pallas as pl
import jax.experimental.pallas.tpu as pltpu

S, D, H, DH, F = 2048, 512, 32, 16, 1792
EPS = 1e-5
QSCALE = (DH ** -0.5) * math.log2(math.e)
L_MIN = 2.0 ** -40
BF = jnp.bfloat16
F32 = jnp.float32
U32 = jnp.uint32


def _pack(x_bf16):
    return pltpu.bitcast(x_bf16, U32)


def _unpack(x_u32):
    return pltpu.bitcast(x_u32, BF)


def _ln(x):
    m = jnp.mean(x, axis=-1, keepdims=True)
    xc = x - m
    v = jnp.mean(xc * xc, axis=-1, keepdims=True)
    return xc * lax.rsqrt(v + EPS)


def make_kernel(TQ=512, KC=128, RC=512, FC=256):
    NQ = S // TQ
    NKC = S // KC

    def kernel(x_ref, wqkv_ref, wo_ref, wg_ref, wu_ref, wd_ref, o_ref,
               k_s, qt_s, vt_s, kmax_s, w_s, pa, pb, ot_s):
        qi = pl.program_id(0)

        @pl.when(qi == 0)
        def _prologue():
            wq_t = wqkv_ref[:, 0:D].T
            wv_t = wqkv_ref[:, 2 * D:3 * D].T
            wqv_t = jnp.concatenate([wq_t, wv_t], axis=0)
            wk = wqkv_ref[:, D:2 * D]
            row = lax.broadcasted_iota(jnp.int32, (H, D), 0)
            col = lax.broadcasted_iota(jnp.int32, (H, D), 1)
            e = jnp.where(col // DH == row, 1.0, 0.0).astype(BF)
            kmax = jnp.zeros((H, RC), F32)
            for r in range(S // RC):
                xn = _ln(x_ref[r * RC:(r + 1) * RC, :].astype(F32)).astype(BF)
                k = jnp.dot(xn, wk, preferred_element_type=F32).astype(BF)
                for g in range(4):
                    k_s[g, r * RC // 2:(r + 1) * RC // 2, :] = _pack(k[:, g * 128:(g + 1) * 128])
                kf = k.astype(F32)
                kk = (kf * kf).astype(BF)
                kn2 = lax.dot_general(e, kk, (((1,), (1,)), ((), ())), preferred_element_type=F32)
                kmax = jnp.maximum(kmax, kn2)
                qv = lax.dot_general(wqv_t, xn, (((1,), (1,)), ((), ())), preferred_element_type=F32)
                qt_s[:, r * RC:(r + 1) * RC] = _pack((qv[:D] * QSCALE).astype(BF))
                vt_s[:, r * RC:(r + 1) * RC] = _pack(qv[D:].astype(BF))
            kmax_s[...] = jnp.broadcast_to(jnp.max(kmax, axis=1, keepdims=True), (H, TQ))
            w_s[...] = jnp.zeros_like(w_s)

        q0 = pl.multiple_of(qi * TQ, TQ)

        def load_w(h):
            hh = h % 8
            r0 = pl.multiple_of(h * 8, 8)
            w0 = pl.multiple_of(hh * 8, 8)
            qh = qt_s[pl.ds(r0, 8), pl.ds(q0, TQ)]
            w_s[pl.ds(w0, 8), :] = qh
            w = _unpack(w_s[...])
            w_s[pl.ds(w0, 8), :] = jnp.zeros((8, TQ), U32)
            return w, _unpack(qh).astype(F32)

        def stage(h, p_new, p_old, l_old, lmin, do_qk, do_pv):
            if do_qk:
                g = h // 8
                w, qf = load_w(h)
                qn2 = jnp.sum(qf * qf, axis=0, keepdims=True)
                m = jnp.sqrt(qn2 * kmax_s[pl.ds(h, 1), :])
                l = jnp.zeros((8, TQ), F32)
            if do_pv:
                r1 = pl.multiple_of((h - 1) * 8, 8)
                acc = jnp.zeros((DH, TQ), F32)
            for c in range(NKC):
                if do_qk:
                    kc = _unpack(k_s[g, c * KC // 2:(c + 1) * KC // 2, :])
                    s = jnp.dot(kc, w, preferred_element_type=F32)
                    p = jnp.exp2(s - m)
                    l = l + jnp.sum(p.reshape(KC // 8, 8, TQ), axis=0)
                    p_new[c * KC // 2:(c + 1) * KC // 2, :] = _pack(p.astype(BF))
                if do_pv:
                    vt = _unpack(vt_s[pl.ds(r1, 8), c * KC:(c + 1) * KC])
                    acc = acc + jnp.dot(vt, _unpack(p_old[c * KC // 2:(c + 1) * KC // 2, :]),
                                        preferred_element_type=F32)
            if do_pv:
                lt = jnp.sum(l_old, axis=0, keepdims=True)
                lmin = jnp.minimum(lmin, lt)
                ot_s[pl.ds(pl.multiple_of((h - 1) * DH, DH), DH), :] = acc / lt
            return (l if do_qk else None), lmin

        lmin = jnp.full((1, TQ), 1.0, F32)
        l, lmin = stage(0, pa, None, None, lmin, True, False)

        def body(i, carry):
            l, lmin = carry
            h = 1 + 2 * i
            l, lmin = stage(h, pb, pa, l, lmin, True, True)
            l, lmin = stage(h + 1, pa, pb, l, lmin, True, True)
            return l, lmin

        l, lmin = lax.fori_loop(0, (H - 2) // 2, body, (l, lmin))
        l, lmin = stage(H - 1, pb, pa, l, lmin, True, True)
        _, lmin = stage(H, None, pb, l, lmin, False, True)

        unsafe = jnp.logical_not(jnp.min(lmin) >= L_MIN)

        @pl.when(unsafe)
        def _fallback():
            def head(h, carry):
                g = h // 8
                w, _ = load_w(h)
                r1 = pl.multiple_of(h * 8, 8)

                def scores(c):
                    c0 = pl.multiple_of(c * 128, 128)
                    kc = _unpack(k_s[g, pl.ds(c0, 128), :])
                    return jnp.dot(kc, w, preferred_element_type=F32)

                def p1(c, m):
                    return jnp.maximum(m, jnp.max(scores(c), axis=0, keepdims=True))

                m = lax.fori_loop(0, S // 256, p1, jnp.full((1, TQ), -jnp.inf, F32))

                def p2(c, carry):
                    l, acc = carry
                    p = jnp.exp2(scores(c) - m)
                    vt = _unpack(vt_s[pl.ds(r1, 8), pl.ds(pl.multiple_of(c * 256, 256), 256)])
                    acc = acc + jnp.dot(vt, p.astype(BF), preferred_element_type=F32)
                    return l + jnp.sum(p, axis=0, keepdims=True), acc

                l, acc = lax.fori_loop(0, S // 256, p2,
                                       (jnp.zeros((1, TQ), F32), jnp.zeros((DH, TQ), F32)))
                ot_s[pl.ds(pl.multiple_of(h * DH, DH), DH), :] = acc / l
                return carry

            lax.fori_loop(0, H, head, 0)

        o = ot_s[...].T.astype(BF)
        x = x_ref[pl.ds(q0, TQ), :].astype(F32)
        h1 = x + jnp.dot(o, wo_ref[...], preferred_element_type=F32)
        hn = _ln(h1).astype(BF)
        y = h1
        for f in range(F // FC):
            gt = jnp.dot(hn, wg_ref[:, f * FC:(f + 1) * FC], preferred_element_type=F32)
            up = jnp.dot(hn, wu_ref[:, f * FC:(f + 1) * FC], preferred_element_type=F32)
            a = (gt * jax.nn.sigmoid(gt) * up).astype(BF)
            y = y + jnp.dot(a, wd_ref[f * FC:(f + 1) * FC, :], preferred_element_type=F32)
        o_ref[...] = y.astype(o_ref.dtype)

    def fn(A_x, A_wqkv, A_wo, B_x, B_w_gate, B_w_up, B_w_down):
        x = A_x.reshape(S, D)
        full = lambda shape: pl.BlockSpec(shape, lambda i: (0,) * len(shape))
        out = pl.pallas_call(
            kernel,
            grid=(NQ,),
            in_specs=[full((S, D)), full((D, 3 * D)), full((D, D)), full((D, F)), full((D, F)), full((F, D))],
            out_specs=pl.BlockSpec((TQ, D), lambda i: (i, 0)),
            out_shape=jax.ShapeDtypeStruct((S, D), BF),
            scratch_shapes=[
                pltpu.VMEM((4, S // 2, 128), U32),
                pltpu.VMEM((D // 2, S), U32),
                pltpu.VMEM((D // 2, S), U32),
                pltpu.VMEM((H, TQ), F32),
                pltpu.VMEM((64, TQ), U32),
                pltpu.VMEM((S // 2, TQ), U32),
                pltpu.VMEM((S // 2, TQ), U32),
                pltpu.VMEM((D, TQ), F32),
            ],
            compiler_params=pltpu.CompilerParams(
                dimension_semantics=("arbitrary",), vmem_limit_bytes=100 * 1024 * 1024),
        )(x, A_wqkv, A_wo, B_w_gate, B_w_up, B_w_down)
        return out.reshape(1, S, D)

    return fn


_impl = make_kernel()


@jax.jit
def pallas_sequential_preLN__softmax_full_mha__swiglu_ffn__prompt_kernel(
    A_x: jax.Array,
    A_wqkv: jax.Array,
    A_wo: jax.Array,
    B_x: jax.Array,
    B_w_gate: jax.Array,
    B_w_up: jax.Array,
    B_w_down: jax.Array,
):
    return _impl(A_x, A_wqkv, A_wo, B_x, B_w_gate, B_w_up, B_w_down)
```

```python
import functools
import math

import jax
import jax.numpy as jnp
from jax import lax
import jax.experimental.pallas as pl
import jax.experimental.pallas.tpu as pltpu

S, D, H, DH, F = 2048, 512, 32, 16, 1792
NV = 5
NM = H - NV
CM = NM * DH
TQ = 512
KC = 128
NKC = S // KC
EPS = 1e-5
QSCALE = (DH ** -0.5) * math.log2(math.e)
L_MIN = 2.0 ** -40
L_MAX = 2.0 ** 40
BF = jnp.bfloat16
F32 = jnp.float32
U32 = jnp.uint32
I32 = jnp.int32
ONES = 0x3F803F80
NT = (((1,), (1,)), ((), ()))


def _pack(x):
    return pltpu.bitcast(x, U32)


def _unpack(x):
    return pltpu.bitcast(x, BF)


def _ln(x):
    m = jnp.mean(x, axis=-1, keepdims=True)
    xc = x - m
    v = jnp.mean(xc * xc, axis=-1, keepdims=True)
    return xc * lax.rsqrt(v + EPS)


def _iota(shape, dim):
    return lax.broadcasted_iota(I32, shape, dim)


def make_kernel(RC=512, FC=256, G=2, J=2, LAG=1, PSPLIT=4, PVMODE=1, HEAD=6, GEND=4, ANCH=2, FORCE_FALLBACK=False):
    NQ = S // TQ
    BPU = (128 // (8 * G)) * (S // (128 * J))
    NJ = S // (128 * J)
    Z_K = 3 * BPU
    Z_P = Z_K + 4
    Z_G = Z_P + 4
    NZ = Z_G + 51
    CPS = NKC // PSPLIT

    def kernel(x_hbm, wqkv_hbm, wo_hbm, wg_hbm, wu_hbm, wd_hbm, o_ref,
               x_ref, wqkv_ref, xn_s, xsem, wo_ref, wg_ref, wu_ref, wd_ref, wsem,
               wn_s, wt_s, kr_s, qt_s, vt_s, vtv_s, qn_s, ktr_s, ktv_s, nq_s, kmx_s, ot_s,
               q0, q1, p0, p1, kA, kB, kC, z_s, l_s, mm_s, *pab):
        step = pl.program_id(0)
        Q = (q0, q1)
        P = (p0, p1)
        KT = (kA, kB, kC)
        PA = pab[:PSPLIT]
        PB = pab[PSPLIT:]

        def wcopies():
            return [pltpu.make_async_copy(src, dst, wsem.at[n]) for n, (src, dst) in enumerate(
                ((wo_hbm, wo_ref), (wg_hbm, wg_ref), (wu_hbm, wu_ref), (wd_hbm, wd_ref)))]

        def xcopy(r):
            return pltpu.make_async_copy(x_hbm.at[pl.ds(r * RC, RC)], x_ref.at[pl.ds(r * RC, RC)], xsem.at[r])

        def wqkv_copy():
            return pltpu.make_async_copy(wqkv_hbm, wqkv_ref, xsem.at[S // RC])

        def unit_calc(a, i):
            u = jnp.minimum(a * NM + i, 16 * NV - 1)
            return lax.shift_right_logical(u, 4), u & 15

        def gen_qb(jt, dst, a, ds, zi=None):
            j, t = jt
            if zi is not None:
                t = t + z_s[zi]
            qn = qn_s[pl.ds(pl.multiple_of(t * 128, 128), 128), :]
            for d in ds:
                lane = (48 + 16 * j + d) if d < 16 else j
                v = jnp.take_along_axis(qn, jnp.full((128, 128), lane, I32), axis=1)
                if d == 16:
                    v = v * kmx_s[pl.ds(NM + j, 1), :]
                dst[a * 17 + d] = v
            return v

        def bias_rows(h):
            nq = nq_s[pl.ds(h, 1), :]
            km = jnp.concatenate([kmx_s[pl.ds(h, 1), :]] * (S // 128), axis=1)
            bits = lax.shift_right_logical(pltpu.bitcast((nq * km).astype(BF).astype(F32), U32), jnp.uint32(16))
            row = pl.multiple_of(h * 16 + 8, 8)
            qt_s[pl.ds(row, 8), :] = jnp.where(_iota((8, S), 0) == 0, jnp.broadcast_to(bits, (8, S)), jnp.uint32(0))

        def vpu_mac(ksrc, qsrc, a, b, zi):
            z = z_s[zi]
            g, j = b // NJ, b % NJ
            acc = jnp.concatenate([qsrc[z + (a * 17 + 16), g * 8 * G:(g + 1) * 8 * G, :]] * J, axis=1)
            for d in range(16):
                qb = jnp.concatenate([qsrc[z + (a * 17 + d), g * 8 * G:(g + 1) * 8 * G, :]] * J, axis=1)
                kt = jnp.concatenate([ksrc[z + d, :, j * 128 * J:(j + 1) * 128 * J]] * G, axis=0)
                acc = acc + qb * kt
            return acc

        def vpu_exp(pdst, a, b, acc):
            g, j = b // NJ, b % NJ
            pdst[a * 64 + g * 4 * G:a * 64 + (g + 1) * 4 * G, j * 128 * J:(j + 1) * 128 * J] = _pack(
                jnp.exp2(acc).astype(BF))

        def vpu_pv_part(jt, psrc, a, c, acc):
            vt = _unpack(vtv_s[pl.ds(pl.multiple_of(jt[0] * 16, 16), 16), c * 128:(c + 1) * 128])
            pp = _unpack(psrc[a * 64:(a + 1) * 64, c * 128:(c + 1) * 128])
            r = lax.dot_general(vt, pp, NT, preferred_element_type=F32)
            return r if acc is None else acc + r

        def vpu_pv_fin(jt, acc, lmn, lmx):
            j, t = jt
            l = acc[16:17, :]
            ot_s[pl.ds(pl.multiple_of((NM + j) * 16, 16), 16),
                 pl.ds(pl.multiple_of(t * 128, 128), 128)] = acc[:16] / l
            return jnp.minimum(lmn, l), jnp.maximum(lmx, l)

        def half(i, par):
            l_old = l_s[...]
            lmn, lmx = mm_s[0:1, :], mm_s[1:2, :]
            lmn2, lmx2 = mm_s[2:3, 0:128], mm_s[3:4, 0:128]
            blocks = [(a, b) for a in range(3) for b in range(BPU)]
            gens = [(a, d) for a in range(3) for d in range(17)]
            nslots = 4 * NKC
            pvq = [(a, q) for a in range(3) for q in range(4)]
            if PVMODE == 0:
                pv_at = {a * NKC + q * 4 + 3: [(a, q)] for a, q in pvq}
            elif PVMODE == 1:
                pv_at = {}
                for n, aq in enumerate(pvq):
                    pv_at.setdefault(min(nslots - 1, (n + 1) * nslots // 12 - 1), []).append(aq)
            else:
                pv_at = {}
                for n, aq in enumerate(pvq):
                    pv_at.setdefault(min(nslots - 1, (n + 1) * 6 - 1), []).append(aq)
            pending = []
            nb_done = 0
            ng_done = 0
            im1 = jnp.maximum(i - 1, 0)
            vaccs = [None] * 3
            gvals = []
            for _ in range(HEAD):
                a, b = blocks[nb_done]
                vpu_exp(P[par], a, b, vpu_mac(KT[a], Q[par], a, b, nb_done))
                nb_done += 1
            for r in range(4):
                p_new, p_old = (PA, PB) if r % 2 == 0 else (PB, PA)
                zk = z_s[Z_K + r]
                qh = qt_s[pl.ds(pl.multiple_of(i * 16, 16), 16), r * TQ:(r + 1) * TQ]
                w = _unpack(jnp.concatenate([qh, jnp.zeros((48, TQ), U32)], axis=0))
                l = jnp.zeros((8, TQ), F32)
                hp = im1 if r == 0 else i
                rp = (r - 1) % 4
                r1 = pl.multiple_of(hp * 8, 8)
                acc = jnp.zeros((DH, TQ), F32)
                zp = pl.multiple_of(z_s[Z_P + r] * 8, 8)
                for c in range(NKC):
                    slot = r * NKC + c
                    want = HEAD + ((len(blocks) - HEAD) * (slot + 1)) // nslots
                    cur = []
                    while nb_done < want:
                        a, b = blocks[nb_done]
                        cur.append((a, b, vpu_mac(KT[a], Q[par], a, b, nb_done)))
                        nb_done += 1
                    pending.append(cur)
                    co = (c % CPS) * KC // 2
                    kc = _unpack(kr_s[i + zk, c * KC // 2:(c + 1) * KC // 2, :])
                    p = jnp.exp2(jnp.dot(kc, w, preferred_element_type=F32))
                    l = l + jnp.sum(p.reshape(KC // 8, 8, TQ), axis=0)
                    p_new[c // CPS][co:co + KC // 2, :] = _pack(p.astype(BF))
                    vt = _unpack(vt_s[pl.ds(r1, 8), c * KC:(c + 1) * KC])
                    acc = acc + jnp.dot(vt, _unpack(p_old[c // CPS][pl.ds(zp + co, KC // 2), :]),
                                        preferred_element_type=F32)
                    for a, q in pv_at.get(slot, ()):
                        jt = unit_calc(a, im1)
                        for cc in range(4 * q, 4 * q + 4):
                            vaccs[a] = vpu_pv_part(jt, P[1 - par], a, cc, vaccs[a])
                        if q == 3:
                            lmn2, lmx2 = vpu_pv_fin(jt, vaccs[a], lmn2, lmx2)
                    wantg = min(len(gens), (len(gens) * (slot + 1)) // (nslots - GEND) + 1)
                    while ng_done < wantg:
                        a, d = gens[ng_done]
                        gv = gen_qb(unit_calc(a, i + 1), Q[1 - par], a, [d], Z_G + ng_done)
                        gvals.append(gv[120:128, :])
                        ng_done += 1
                    while ANCH and len(gvals) > ANCH:
                        one = jnp.exp2(gvals.pop(0) * 0.0)
                        l = jnp.concatenate([l[:, :128] * one, l[:, 128:]], axis=1)
                    while len(pending) > LAG:
                        for a, b, ac in pending.pop(0):
                            vpu_exp(P[par], a, b, ac)
                lt = jnp.sum(l_old, axis=0, keepdims=True)
                lmn, lmx = jnp.minimum(lmn, lt), jnp.maximum(lmx, lt)
                ot_s[pl.ds(pl.multiple_of(hp * 16, 16), DH), rp * TQ:(rp + 1) * TQ] = acc / lt
                l_old = l
            while pending:
                for a, b, ac in pending.pop(0):
                    vpu_exp(P[par], a, b, ac)
            bias_rows(jnp.minimum(i + 1, NM - 1))
            l_s[...] = l_old
            mm_s[0:1, :] = lmn
            mm_s[1:2, :] = lmx
            mm_s[2:3, 0:128] = lmn2
            mm_s[3:4, 0:128] = lmx2

        def kt_update(i):
            for a, kd in enumerate(KT):
                j, t = unit_calc(a, i)

                @pl.when(jnp.logical_or(t == 0, i == 0))
                def _():
                    def cp(d, c):
                        kd[d] = ktr_s[j * 16 + d]
                        return c
                    lax.fori_loop(0, 16, cp, 0)

        def prologue():
            for b in range(NZ):
                z_s[b] = 0

            def ln1(r, c):
                xcopy(r).wait()
                rows = pl.ds(pl.multiple_of(r * RC, RC), RC)
                prow = pl.ds(pl.multiple_of(r * (RC // 2), RC // 2), RC // 2)
                xn_s[prow, :] = _pack(_ln(x_ref[rows, :].astype(F32)).astype(BF))
                return c

            lax.fori_loop(0, S // RC, ln1, 0)
            wqkv_copy().wait()
            for cp in wcopies():
                cp.start()
            col = _iota((D, D), 1)
            wq = wqkv_ref[:, 0:D]
            wk = wqkv_ref[:, D:2 * D]
            wn_s[...] = _pack(jnp.where(col < CM, wk, wq))
            wt_s[0:D // 2, :] = _pack(jnp.where(col < CM, wq, wk).T)
            wt_s[D // 2:D, :] = _pack(wqkv_ref[:, 2 * D:3 * D].T)

            def chunk(r, kmax):
                e = jnp.where(_iota((H, D), 1) // DH == _iota((H, D), 0), 1.0, 0.0).astype(BF)
                e2r = _iota((128, 128), 0)
                e2 = jnp.where((e2r >= 48) & ((e2r - 48) // DH == _iota((128, 128), 1)), 1.0, 0.0).astype(BF)
                lane_k = _iota((RC // 2, 128), 1)
                lane_q = _iota((RC, 128), 1)
                kfill = jnp.where(lane_k == DH, ONES, 0).astype(U32)
                rscale = jnp.where(_iota((D, RC), 0) < CM, QSCALE, 1.0).astype(F32)
                onesblk = jnp.where(_iota((8, RC), 0) == 0, 0x00003F80, 0).astype(U32)
                rows = pl.ds(pl.multiple_of(r * RC, RC), RC)
                prow = pl.ds(pl.multiple_of(r * (RC // 2), RC // 2), RC // 2)
                xn = _unpack(xn_s[prow, :])
                kn = jnp.dot(xn, _unpack(wn_s[...]), preferred_element_type=F32)
                kb = kn.astype(BF)
                kp = _pack(kb)
                for h in range(NM):
                    g, hh = h // 8, h % 8
                    kg = kp[:, g * 128:(g + 1) * 128]
                    if hh:
                        kg = pltpu.roll(kg, 128 - DH * hh, 1)
                    kr_s[h, prow, :] = jnp.where(lane_k < DH, kg, kfill)
                kf = kb.astype(F32)
                kn2 = lax.dot_general(e, (kf * kf).astype(BF), NT, preferred_element_type=F32)
                qv = kn[:, 384:512] * QSCALE
                qv2 = jnp.dot((qv * qv).astype(BF), e2, preferred_element_type=F32)
                qn_s[rows, :] = jnp.where(lane_q < 48, jnp.sqrt(qv2), qv)
                t = lax.dot_general(_unpack(wt_s[...]), xn, NT, preferred_element_type=F32)
                tqk = t[:D] * rscale
                tb = tqk.astype(BF)
                tp = _pack(tb)
                for h in range(NM):
                    qt_s[h * 16:h * 16 + 8, rows] = tp[h * 8:(h + 1) * 8]
                ktv_s[24:64, rows] = tp[CM // 2:]
                for rr in range(NV * DH):
                    ktr_s[rr, :, rows] = jnp.broadcast_to(tqk[CM + rr:CM + rr + 1, :], (8, RC))
                tf = tb.astype(F32)
                n2 = jnp.dot(e, (tf * tf).astype(BF), preferred_element_type=F32)
                nq_s[:, rows] = jnp.sqrt(n2)
                kmax = jnp.maximum(kmax, jnp.where(_iota((H, RC), 0) < NM, kn2, n2))
                vp = _pack(t[D:].astype(BF))
                vt_s[:, rows] = vp[:CM // 2]
                for j in range(NV):
                    vtv_s[j * 16:j * 16 + 8, rows] = vp[CM // 2 + j * 8:CM // 2 + (j + 1) * 8]
                    vtv_s[j * 16 + 8:j * 16 + 16, rows] = onesblk
                pr = pl.ds(pl.multiple_of(r * (RC // 2 // PSPLIT), 8), RC // 2 // PSPLIT)
                for pp in PB:
                    pp[pr, :] = jnp.full((RC // 2 // PSPLIT, TQ), ONES, U32)
                p1[:, rows] = jnp.full((192, RC), ONES, U32)
                ktv_s[0:24, rows] = jnp.zeros((24, RC), U32)
                a = (2 * r) % 3
                gen_qb(unit_calc(a, 0), q0, a, list(range(16)))
                return kmax

            kmax = lax.fori_loop(0, S // RC, chunk, jnp.zeros((H, RC), F32))
            kmx_s[...] = jnp.broadcast_to(-jnp.sqrt(jnp.max(kmax, axis=1, keepdims=True)), (H, 128))
            bias_rows(0)
            l_s[...] = jnp.ones(l_s.shape, F32)
            mm_s[...] = jnp.ones(mm_s.shape, F32)
            for a in range(3):
                gen_qb(unit_calc(a, jnp.int32(0)), q0, a, [16])

        def attention():
            def body(ii, carry):
                i = 2 * ii
                kt_update(i)
                half(i, 0)

                @pl.when(i + 1 < NM)
                def _():
                    kt_update(i + 1)
                    half(i + 1, 1)
                return carry

            lax.fori_loop(0, (NM + 1) // 2, body, 0)
            lmn, lmx = mm_s[0:1, :], mm_s[1:2, :]
            lmn2, lmx2 = mm_s[2:3, 0:128], mm_s[3:4, 0:128]
            hp = NM - 1
            pw = jnp.concatenate([pp[...] for pp in PB], axis=0)
            acc = jnp.dot(_unpack(vt_s[hp * 8:(hp + 1) * 8, :]), _unpack(pw), preferred_element_type=F32)
            lt = jnp.sum(l_s[...], axis=0, keepdims=True)
            lmn, lmx = jnp.minimum(lmn, lt), jnp.maximum(lmx, lt)
            ot_s[hp * 16:(hp + 1) * 16, 3 * TQ:] = acc / lt
            for a in range(3):
                vacc = None
                jt = unit_calc(a, jnp.int32(NM - 1))
                for cc in range(16):
                    vacc = vpu_pv_part(jt, P[(NM - 1) % 2], a, cc, vacc)
                lmn2, lmx2 = vpu_pv_fin(jt, vacc, lmn2, lmx2)
            lo = jnp.minimum(jnp.min(lmn), jnp.min(lmn2))
            hi = jnp.maximum(jnp.max(lmx), jnp.max(lmx2))
            return jnp.logical_not(jnp.logical_and(lo >= L_MIN, hi <= L_MAX))

        def fallback():
            def mxu_item(n, carry):
                h = lax.shift_right_logical(n, 3)
                c0 = pl.multiple_of((n & 7) * 256, 256)
                qh = qt_s[pl.ds(pl.multiple_of(h * 16, 16), 8), pl.ds(c0, 256)]
                w = _unpack(jnp.concatenate([qh, jnp.zeros((56, 256), U32)], axis=0))

                def scores(c):
                    kc = _unpack(kr_s[h, pl.ds(pl.multiple_of(c * 64, 64), 64), :])
                    return jnp.dot(kc, w, preferred_element_type=F32)

                m = lax.fori_loop(
                    0, S // 128,
                    lambda c, m: jnp.maximum(m, jnp.max(scores(c), axis=0, keepdims=True)),
                    jnp.full((1, 256), -jnp.inf, F32))

                def p2(c, carry):
                    l, acc = carry
                    p = jnp.exp2(scores(c) - m)
                    vt = _unpack(vt_s[pl.ds(pl.multiple_of(h * 8, 8), 8), pl.ds(pl.multiple_of(c * 128, 128), 128)])
                    acc = acc + jnp.dot(vt, p.astype(BF), preferred_element_type=F32)
                    return l + jnp.sum(p, axis=0, keepdims=True), acc

                l, acc = lax.fori_loop(0, S // 128, p2, (jnp.zeros((1, 256), F32), jnp.zeros((DH, 256), F32)))
                ot_s[pl.ds(pl.multiple_of(h * DH, DH), DH), pl.ds(c0, 256)] = acc / l
                return carry

            lax.fori_loop(0, NM * 8, mxu_item, 0)

            def vpu_item(u, carry):
                j = lax.shift_right_logical(u, 4)
                t0 = pl.multiple_of((u & 15) * 128, 128)
                lane = _iota((128, 128), 1)
                lo = 48 + 16 * j
                qm = jnp.where((lane >= lo) & (lane < lo + DH), qn_s[pl.ds(t0, 128), :], 0.0).astype(BF)

                def scores(c):
                    kt = _unpack(ktv_s[:, pl.ds(pl.multiple_of(c * 128, 128), 128)])
                    return jnp.dot(qm, kt, preferred_element_type=F32)

                m = lax.fori_loop(0, S // 128, lambda c, m: jnp.maximum(m, scores(c)),
                                  jnp.full((128, 128), -jnp.inf, F32))
                m = jnp.max(m, axis=1, keepdims=True)

                def p2(c, acc):
                    p = jnp.exp2(scores(c) - m).astype(BF)
                    vt = _unpack(vtv_s[pl.ds(pl.multiple_of(j * 16, 16), 16), pl.ds(pl.multiple_of(c * 128, 128), 128)])
                    return acc + lax.dot_general(vt, p, NT, preferred_element_type=F32)

                acc = lax.fori_loop(0, S // 128, p2, jnp.zeros((32, 128), F32))
                ot_s[pl.ds(pl.multiple_of((NM + j) * 16, 16), 16), pl.ds(t0, 128)] = acc[:16] / acc[16:17]
                return carry

            lax.fori_loop(0, NV * 16, vpu_item, 0)

        @pl.when(step == 0)
        def _():
            for r in range(S // RC):
                xcopy(r).start()
            wqkv_copy().start()
            prologue()
            unsafe = attention()
            if FORCE_FALLBACK:
                unsafe = step == 0
            pl.when(unsafe)(fallback)
            for cp in wcopies():
                cp.wait()

        c0 = pl.multiple_of(step * TQ, TQ)
        o = ot_s[:, pl.ds(c0, TQ)].T.astype(BF)
        x = x_ref[pl.ds(c0, TQ), :].astype(F32)
        h1 = x + jnp.dot(o, wo_ref[...], preferred_element_type=F32)
        hn = _ln(h1).astype(BF)
        y = h1
        for f in range(F // FC):
            gt = jnp.dot(hn, wg_ref[:, f * FC:(f + 1) * FC], preferred_element_type=F32)
            up = jnp.dot(hn, wu_ref[:, f * FC:(f + 1) * FC], preferred_element_type=F32)
            a = (gt * jax.nn.sigmoid(gt) * up).astype(BF)
            y = y + jnp.dot(a, wd_ref[f * FC:(f + 1) * FC, :], preferred_element_type=F32)
        o_ref[...] = y.astype(o_ref.dtype)

    def fn(A_x, A_wqkv, A_wo, B_x, B_w_gate, B_w_up, B_w_down):
        x = A_x.reshape(S, D)
        hbm = pl.BlockSpec(memory_space=pl.ANY)
        out = pl.pallas_call(
            kernel,
            grid=(NQ,),
            in_specs=[hbm] * 6,
            out_specs=pl.BlockSpec((TQ, D), lambda i: (i, 0)),
            out_shape=jax.ShapeDtypeStruct((S, D), BF),
            scratch_shapes=[
                pltpu.VMEM((S, D), BF), pltpu.VMEM((D, 3 * D), BF), pltpu.VMEM((S // 2, D), U32),
                pltpu.SemaphoreType.DMA((S // RC + 1,)),
                pltpu.VMEM((D, D), BF), pltpu.VMEM((D, F), BF), pltpu.VMEM((D, F), BF), pltpu.VMEM((F, D), BF),
                pltpu.SemaphoreType.DMA((4,)),
                pltpu.VMEM((D // 2, D), U32), pltpu.VMEM((D, D), U32),
                pltpu.VMEM((NM, S // 2, 128), U32),
                pltpu.VMEM((NM * 16, S), U32),
                pltpu.VMEM((NM * 8, S), U32),
                pltpu.VMEM((NV * 16, S), U32),
                pltpu.VMEM((S, 128), F32),
                pltpu.VMEM((NV * 16, 8, S), F32),
                pltpu.VMEM((64, S), U32),
                pltpu.VMEM((H, S), F32),
                pltpu.VMEM((H, 128), F32),
                pltpu.VMEM((D, S), F32)]
                + [pltpu.VMEM((51, 128, 128), F32)] * 2
                + [pltpu.VMEM((192, S), U32)] * 2
                + [pltpu.VMEM((16, 8, S), F32)] * 3
                + [pltpu.SMEM((NZ,), I32), pltpu.VMEM((8, TQ), F32), pltpu.VMEM((8, TQ), F32)]
                + [pltpu.VMEM((S // 2 // PSPLIT, TQ), U32)] * (2 * PSPLIT),
            compiler_params=pltpu.CompilerParams(
                dimension_semantics=("arbitrary",), vmem_limit_bytes=110 * 1024 * 1024),
        )(x, A_wqkv, A_wo, B_w_gate, B_w_up, B_w_down)
        return out.reshape(1, S, D)

    return fn


_impl = make_kernel()


@jax.jit
def pallas_sequential_preLN__softmax_full_mha__swiglu_ffn__prompt_kernel(
    A_x: jax.Array,
    A_wqkv: jax.Array,
    A_wo: jax.Array,
    B_x: jax.Array,
    B_w_gate: jax.Array,
    B_w_up: jax.Array,
    B_w_down: jax.Array,
):
    return _impl(A_x, A_wqkv, A_wo, B_x, B_w_gate, B_w_up, B_w_down)
```

```python
import functools
import math

import jax
import jax.numpy as jnp
from jax import lax
import jax.experimental.pallas as pl
import jax.experimental.pallas.tpu as pltpu

S, D, H, DH, F = 2048, 512, 32, 16, 1792
NV = 5
NM = H - NV
CM = NM * DH
TQ = 512
KC = 128
NKC = S // KC
EPS = 1e-5
QSCALE = (DH ** -0.5) * math.log2(math.e)
L_MIN = 2.0 ** -40
L_MAX = 2.0 ** 40
BF = jnp.bfloat16
F32 = jnp.float32
U32 = jnp.uint32
I32 = jnp.int32
ONES = 0x3F803F80
NT = (((1,), (1,)), ((), ()))


def _pack(x):
    return pltpu.bitcast(x, U32)


def _unpack(x):
    return pltpu.bitcast(x, BF)


def _ln(x):
    m = jnp.mean(x, axis=-1, keepdims=True)
    xc = x - m
    v = jnp.mean(xc * xc, axis=-1, keepdims=True)
    return xc * lax.rsqrt(v + EPS)


def _iota(shape, dim):
    return lax.broadcasted_iota(I32, shape, dim)


def make_kernel(RC=512, FC=256, G=2, J=2, LAG=3, PSPLIT=4, HEAD=6, GEND=4, ANCH=2, NTP=8, LNP=(3, 4, 5, 6),
                TD=512, PVLAG=0, VEND=0, FORCE_FALLBACK=False):
    NQ = S // TD
    BPU = (128 // (8 * G)) * (S // (128 * J))
    NJ = S // (128 * J)
    Z_K = 3 * BPU
    Z_P = Z_K + 4
    Z_G = Z_P + 4
    Z_T = Z_G + 51
    NZ = Z_T
    CPS = NKC // PSPLIT

    def kernel(x_hbm, wqkv_hbm, wo_hbm, wg_hbm, wu_hbm, wd_hbm, o_ref,
               x_ref, wqkv_ref, xsem, wo_ref, wg_ref, wu_ref, wd_ref, wsem,
               wn_s, wt_s, kr_s, qt_s, vt_s, vtv_s, qn_s, ktr_s, ktv_s, nq_s, kmx_s, ot_s,
               q0, q1, p0, p1, z_s, l_s, mm_s, *pab):
        step = pl.program_id(0)
        Q = (q0, q1)
        P = (p0, p1)
        PA = pab[:PSPLIT]
        PB = pab[PSPLIT:]

        def wcopies():
            return [pltpu.make_async_copy(src, dst, wsem.at[n]) for n, (src, dst) in enumerate(
                ((wo_hbm, wo_ref), (wg_hbm, wg_ref), (wu_hbm, wu_ref), (wd_hbm, wd_ref)))]

        def xcopy(r):
            return pltpu.make_async_copy(x_hbm.at[pl.ds(r * RC, RC)], x_ref.at[pl.ds(r * RC, RC)], xsem.at[r])

        def wqkv_copy():
            return pltpu.make_async_copy(wqkv_hbm, wqkv_ref, xsem.at[S // RC])

        def unit_calc(a, i):
            u = jnp.minimum(a * NM + i, 16 * NV - 1)
            return lax.shift_right_logical(u, 4), u & 15

        def gen_qb(jt, dst, a, ds, zi=None):
            j, t = jt
            if zi is not None:
                t = t + z_s[zi]
            qn = qn_s[pl.ds(pl.multiple_of(t * 128, 128), 128), :]
            for d in ds:
                lane = (48 + 16 * j + d) if d < 16 else j
                v = jnp.take_along_axis(qn, jnp.full((128, 128), lane, I32), axis=1)
                if d == 16:
                    v = v * kmx_s[pl.ds(NM + j, 1), :]
                dst[a * 17 + d] = v
            return v

        def bias_rows(h):
            nq = nq_s[pl.ds(h, 1), :]
            km = jnp.concatenate([kmx_s[pl.ds(h, 1), :]] * (S // 128), axis=1)
            bits = lax.shift_right_logical(pltpu.bitcast((nq * km).astype(BF).astype(F32), U32), jnp.uint32(16))
            row = pl.multiple_of(h * 16 + 8, 8)
            qt_s[pl.ds(row, 8), :] = jnp.where(_iota((8, S), 0) == 0, jnp.broadcast_to(bits, (8, S)), jnp.uint32(0))

        def vpu_mac(par, qsrc, a, b, zi):
            z = z_s[zi]
            zk = z_s[Z_T + par * 3 * BPU + zi]
            g, j = b // NJ, b % NJ
            acc = jnp.concatenate([qsrc[z + (a * 17 + 16), g * 8 * G:(g + 1) * 8 * G, :]] * J, axis=1)
            for d in range(16):
                qb = jnp.concatenate([qsrc[z + (a * 17 + d), g * 8 * G:(g + 1) * 8 * G, :]] * J, axis=1)
                kt = jnp.concatenate([ktr_s[zk + d, :, j * 128 * J:(j + 1) * 128 * J]] * G, axis=0)
                acc = acc + qb * kt
            return acc

        def vpu_exp(pdst, a, b, acc):
            g, j = b // NJ, b % NJ
            pdst[a * 64 + g * 4 * G:a * 64 + (g + 1) * 4 * G, j * 128 * J:(j + 1) * 128 * J] = _pack(
                jnp.exp2(acc).astype(BF))

        def vpu_pv_part(jt, psrc, a, c, acc):
            vt = _unpack(vtv_s[pl.ds(pl.multiple_of(jt[0] * 16, 16), 16), c * 128:(c + 1) * 128])
            pp = _unpack(psrc[a * 64:(a + 1) * 64, c * 128:(c + 1) * 128])
            r = lax.dot_general(vt, pp, NT, preferred_element_type=F32)
            return r if acc is None else acc + r

        def vpu_pv_fin(jt, acc, lmn, lmx):
            j, t = jt
            l = acc[16:17, :]
            ot_s[pl.ds(pl.multiple_of((NM + j) * 16, 16), 16),
                 pl.ds(pl.multiple_of(t * 128, 128), 128)] = acc[:16] / l
            return jnp.minimum(lmn, l), jnp.maximum(lmx, l)

        def half(i, par):
            lmn, lmx = mm_s[0:1, :], mm_s[1:2, :]
            lmn2, lmx2 = mm_s[2:3, 0:128], mm_s[3:4, 0:128]
            blocks = [(a, b) for a in range(3) for b in range(BPU)]
            gens = [(a, d) for a in range(3) for d in range(17)]
            nslots = 4 * NKC
            pv_at = {}
            for n in range(12):
                pv_at.setdefault((n + 1) * (nslots - VEND) // 12 - 1, []).append((n // 4, n % 4))
            im1 = jnp.maximum(i - 1, 0)
            pending, gvals = [], []
            nb_done = ng_done = npv_done = 0
            vaccs = [None] * 3
            accs = [None] * 4
            ls = [l_s[...]] + [jnp.zeros((8, TQ), F32) for _ in range(4)]
            for _ in range(HEAD):
                a, b = blocks[nb_done]
                vpu_exp(P[par], a, b, vpu_mac(par, Q[par], a, b, nb_done))
                nb_done += 1
            for slot in range(nslots):
                r, c = slot // NKC, slot % NKC
                want = HEAD + ((len(blocks) - HEAD) * (slot + 1)) // nslots
                while nb_done < want:
                    a, b = blocks[nb_done]
                    pending.append((a, b, vpu_mac(par, Q[par], a, b, nb_done)))
                    nb_done += 1
                if c == 0:
                    zk = z_s[Z_K + r]
                    qh = qt_s[pl.ds(pl.multiple_of(i * 16, 16), 16), r * TQ:(r + 1) * TQ]
                    w = _unpack(jnp.concatenate([qh, jnp.zeros((48, TQ), U32)], axis=0))
                kc = _unpack(kr_s[i + zk, c * KC // 2:(c + 1) * KC // 2, :])
                p = jnp.exp2(jnp.dot(kc, w, preferred_element_type=F32))
                ls[r + 1] = ls[r + 1] + jnp.sum(p.reshape(KC // 8, 8, TQ), axis=0)
                co = (c % CPS) * KC // 2
                (PA if r % 2 == 0 else PB)[c // CPS][co:co + KC // 2, :] = _pack(p.astype(BF))
                while npv_done < nslots and (npv_done + PVLAG <= slot or slot == nslots - 1):
                    r2, c2 = npv_done // NKC, npv_done % NKC
                    hp = im1 if r2 == 0 else i
                    zp = pl.multiple_of(z_s[Z_P + r2] * 8, 8)
                    co2 = (c2 % CPS) * KC // 2
                    vt = _unpack(vt_s[pl.ds(pl.multiple_of(hp * 8, 8), 8), c2 * KC:(c2 + 1) * KC])
                    pr = jnp.dot(vt, _unpack((PB if r2 % 2 == 0 else PA)[c2 // CPS][pl.ds(zp + co2, KC // 2), :]),
                                 preferred_element_type=F32)
                    accs[r2] = pr if c2 == 0 else accs[r2] + pr
                    if c2 == NKC - 1:
                        lt = jnp.sum(ls[r2], axis=0, keepdims=True)
                        lmn, lmx = jnp.minimum(lmn, lt), jnp.maximum(lmx, lt)
                        rp = (r2 - 1) % 4
                        ot_s[pl.ds(pl.multiple_of(hp * 16, 16), DH), rp * TQ:(rp + 1) * TQ] = accs[r2] / lt
                    npv_done += 1
                for a, q in pv_at.get(slot, ()):
                    jt = unit_calc(a, im1)
                    for cc in range(4 * q, 4 * q + 4):
                        vaccs[a] = vpu_pv_part(jt, P[1 - par], a, cc, vaccs[a])
                    if q == 3:
                        lmn2, lmx2 = vpu_pv_fin(jt, vaccs[a], lmn2, lmx2)
                wantg = min(len(gens), (len(gens) * (slot + 1)) // (nslots - GEND) + 1)
                while ng_done < wantg:
                    a, d = gens[ng_done]
                    gv = gen_qb(unit_calc(a, i + 1), Q[1 - par], a, [d], Z_G + ng_done)
                    gvals.append(gv[120:128, :])
                    ng_done += 1
                while len(gvals) > ANCH:
                    one = jnp.exp2(gvals.pop(0) * 0.0)
                    ls[r + 1] = jnp.concatenate([ls[r + 1][:, :128] * one, ls[r + 1][:, 128:]], axis=1)
                while len(pending) > (LAG if slot < nslots - 1 else 0):
                    a, b, ac = pending.pop(0)
                    vpu_exp(P[par], a, b, ac)
            bias_rows(jnp.minimum(i + 1, NM - 1))
            set_ktab(i + 1, 1 - par)
            l_s[...] = ls[4]
            mm_s[0:1, :] = lmn
            mm_s[1:2, :] = lmx
            mm_s[2:3, 0:128] = lmn2
            mm_s[3:4, 0:128] = lmx2

        def set_ktab(i, par):
            for a in range(3):
                v = unit_calc(a, i)[0] * 16
                for b in range(BPU):
                    z_s[Z_T + (par * 3 + a) * BPU + b] = v

        def prologue():
            for b in range(NZ):
                z_s[b] = 0

            def ln1(r, n=0, parts=1):
                pr = RC // parts
                rows = pl.ds(pl.multiple_of(r * RC + n * pr, pr), pr)
                return _pack(_ln(x_ref[rows, :].astype(F32)).astype(BF))

            set_ktab(jnp.int32(0), 0)
            xcopy(0).wait()
            xp0 = ln1(0)
            wqkv_copy().wait()
            for cp in wcopies():
                cp.start()
            col = _iota((D, D), 1)
            wq = wqkv_ref[:, 0:D]
            wk = wqkv_ref[:, D:2 * D]
            wn_s[...] = _pack(jnp.where(col < CM, wk, wq))
            wt_s[0:D // 2, :] = _pack(jnp.where(col < CM, wq, wk).T)
            wt_s[D // 2:D, :] = _pack(wqkv_ref[:, 2 * D:3 * D].T)

            def chunk(r, carry):
                kmax, xp = carry
                rn = jnp.minimum(r + 1, S // RC - 1)

                @pl.when(r + 1 < S // RC)
                def _():
                    xcopy(rn).wait()

                e = jnp.where(_iota((H, D), 1) // DH == _iota((H, D), 0), 1.0, 0.0).astype(BF)
                e2r = _iota((128, 128), 0)
                e2 = jnp.where((e2r >= 48) & ((e2r - 48) // DH == _iota((128, 128), 1)), 1.0, 0.0).astype(BF)
                lane_k = _iota((RC // 2, 128), 1)
                lane_q = _iota((RC, 128), 1)
                kfill = jnp.where(lane_k == DH, ONES, 0).astype(U32)
                rscale = jnp.where(_iota((D, RC), 0) < CM, QSCALE, 1.0).astype(F32)
                onesblk = jnp.where(_iota((8, RC), 0) == 0, 0x00003F80, 0).astype(U32)
                rows = pl.ds(pl.multiple_of(r * RC, RC), RC)
                prow = pl.ds(pl.multiple_of(r * (RC // 2), RC // 2), RC // 2)
                xn = _unpack(xp)
                kn = jnp.dot(xn, _unpack(wn_s[...]), preferred_element_type=F32)
                kb = kn.astype(BF)
                kp = _pack(kb)
                for h in range(NM):
                    g, hh = h // 8, h % 8
                    kg = kp[:, g * 128:(g + 1) * 128]
                    if hh:
                        kg = pltpu.roll(kg, 128 - DH * hh, 1)
                    kr_s[h, prow, :] = jnp.where(lane_k < DH, kg, kfill)
                kf = kb.astype(F32)
                kn2 = lax.dot_general(e, (kf * kf).astype(BF), NT, preferred_element_type=F32)
                qv = kn[:, 384:512] * QSCALE
                qv2 = jnp.dot((qv * qv).astype(BF), e2, preferred_element_type=F32)
                qn_s[rows, :] = jnp.where(lane_q < 48, jnp.sqrt(qv2), qv)
                ts, xs = [], []
                for n in range(NTP):
                    wrows = slice(n * D // NTP, (n + 1) * D // NTP)
                    ts.append(lax.dot_general(_unpack(wt_s[wrows, :]), xn, NT, preferred_element_type=F32))
                    for _ in range(LNP.count(n)):
                        xs.append(ln1(rn, len(xs), len(LNP)))
                t = jnp.concatenate(ts, axis=0)
                xp_next = jnp.concatenate(xs, axis=0)
                tqk = t[:D] * rscale
                tb = tqk.astype(BF)
                tp = _pack(tb)
                for h in range(NM):
                    qt_s[h * 16:h * 16 + 8, rows] = tp[h * 8:(h + 1) * 8]
                ktv_s[24:64, rows] = tp[CM // 2:]
                for rr in range(NV * DH):
                    ktr_s[rr, :, rows] = jnp.broadcast_to(tqk[CM + rr:CM + rr + 1, :], (8, RC))
                tf = tb.astype(F32)
                n2 = jnp.dot(e, (tf * tf).astype(BF), preferred_element_type=F32)
                nq_s[:, rows] = jnp.sqrt(n2)
                kmax = jnp.maximum(kmax, jnp.where(_iota((H, RC), 0) < NM, kn2, n2))
                vp = _pack(t[D:].astype(BF))
                vt_s[:, rows] = vp[:CM // 2]
                for j in range(NV):
                    vtv_s[j * 16:j * 16 + 8, rows] = vp[CM // 2 + j * 8:CM // 2 + (j + 1) * 8]
                    vtv_s[j * 16 + 8:j * 16 + 16, rows] = onesblk
                pr = pl.ds(pl.multiple_of(r * (RC // 2 // PSPLIT), 8), RC // 2 // PSPLIT)
                for pp in PB:
                    pp[pr, :] = jnp.full((RC // 2 // PSPLIT, TQ), ONES, U32)
                p1[:, rows] = jnp.full((192, RC), ONES, U32)
                ktv_s[0:24, rows] = jnp.zeros((24, RC), U32)
                a = (2 * r) % 3
                gen_qb(unit_calc(a, 0), q0, a, list(range(16)))
                return kmax, xp_next

            kmax, _ = lax.fori_loop(0, S // RC, chunk, (jnp.zeros((H, RC), F32), xp0))
            kmx_s[...] = jnp.broadcast_to(-jnp.sqrt(jnp.max(kmax, axis=1, keepdims=True)), (H, 128))
            bias_rows(0)
            l_s[...] = jnp.ones(l_s.shape, F32)
            mm_s[...] = jnp.ones(mm_s.shape, F32)
            for a in range(3):
                gen_qb(unit_calc(a, jnp.int32(0)), q0, a, [16])

        def attention():
            def body(ii, carry):
                i = 2 * ii
                half(i, 0)

                @pl.when(i + 1 < NM)
                def _():
                    half(i + 1, 1)
                return carry

            lax.fori_loop(0, (NM + 1) // 2, body, 0)
            lmn, lmx = mm_s[0:1, :], mm_s[1:2, :]
            lmn2, lmx2 = mm_s[2:3, 0:128], mm_s[3:4, 0:128]
            hp = NM - 1
            pw = jnp.concatenate([pp[...] for pp in PB], axis=0)
            acc = jnp.dot(_unpack(vt_s[hp * 8:(hp + 1) * 8, :]), _unpack(pw), preferred_element_type=F32)
            lt = jnp.sum(l_s[...], axis=0, keepdims=True)
            lmn, lmx = jnp.minimum(lmn, lt), jnp.maximum(lmx, lt)
            ot_s[hp * 16:(hp + 1) * 16, 3 * TQ:] = acc / lt
            for a in range(3):
                if a * NM + NM - 1 >= 16 * NV:
                    continue
                vacc = None
                jt = unit_calc(a, jnp.int32(NM - 1))
                for cc in range(16):
                    vacc = vpu_pv_part(jt, P[(NM - 1) % 2], a, cc, vacc)
                lmn2, lmx2 = vpu_pv_fin(jt, vacc, lmn2, lmx2)
            lo = jnp.minimum(jnp.min(lmn), jnp.min(lmn2))
            hi = jnp.maximum(jnp.max(lmx), jnp.max(lmx2))
            return jnp.logical_not(jnp.logical_and(lo >= L_MIN, hi <= L_MAX))

        def fallback():
            def mxu_item(n, carry):
                h = lax.shift_right_logical(n, 3)
                c0 = pl.multiple_of((n & 7) * 256, 256)
                qh = qt_s[pl.ds(pl.multiple_of(h * 16, 16), 8), pl.ds(c0, 256)]
                w = _unpack(jnp.concatenate([qh, jnp.zeros((56, 256), U32)], axis=0))

                def scores(c):
                    kc = _unpack(kr_s[h, pl.ds(pl.multiple_of(c * 64, 64), 64), :])
                    return jnp.dot(kc, w, preferred_element_type=F32)

                m = lax.fori_loop(
                    0, S // 128,
                    lambda c, m: jnp.maximum(m, jnp.max(scores(c), axis=0, keepdims=True)),
                    jnp.full((1, 256), -jnp.inf, F32))

                def p2(c, carry):
                    l, acc = carry
                    p = jnp.exp2(scores(c) - m)
                    vt = _unpack(vt_s[pl.ds(pl.multiple_of(h * 8, 8), 8), pl.ds(pl.multiple_of(c * 128, 128), 128)])
                    acc = acc + jnp.dot(vt, p.astype(BF), preferred_element_type=F32)
                    return l + jnp.sum(p, axis=0, keepdims=True), acc

                l, acc = lax.fori_loop(0, S // 128, p2, (jnp.zeros((1, 256), F32), jnp.zeros((DH, 256), F32)))
                ot_s[pl.ds(pl.multiple_of(h * DH, DH), DH), pl.ds(c0, 256)] = acc / l
                return carry

            lax.fori_loop(0, NM * 8, mxu_item, 0)

            def vpu_item(u, carry):
                j = lax.shift_right_logical(u, 4)
                t0 = pl.multiple_of((u & 15) * 128, 128)
                lane = _iota((128, 128), 1)
                lo = 48 + 16 * j
                qm = jnp.where((lane >= lo) & (lane < lo + DH), qn_s[pl.ds(t0, 128), :], 0.0).astype(BF)

                def scores(c):
                    kt = _unpack(ktv_s[:, pl.ds(pl.multiple_of(c * 128, 128), 128)])
                    return jnp.dot(qm, kt, preferred_element_type=F32)

                m = lax.fori_loop(0, S // 128, lambda c, m: jnp.maximum(m, scores(c)),
                                  jnp.full((128, 128), -jnp.inf, F32))
                m = jnp.max(m, axis=1, keepdims=True)

                def p2(c, acc):
                    p = jnp.exp2(scores(c) - m).astype(BF)
                    vt = _unpack(vtv_s[pl.ds(pl.multiple_of(j * 16, 16), 16), pl.ds(pl.multiple_of(c * 128, 128), 128)])
                    return acc + lax.dot_general(vt, p, NT, preferred_element_type=F32)

                acc = lax.fori_loop(0, S // 128, p2, jnp.zeros((32, 128), F32))
                ot_s[pl.ds(pl.multiple_of((NM + j) * 16, 16), 16), pl.ds(t0, 128)] = acc[:16] / acc[16:17]
                return carry

            lax.fori_loop(0, NV * 16, vpu_item, 0)

        @pl.when(step == 0)
        def _():
            xcopy(0).start()
            wqkv_copy().start()
            for r in range(1, S // RC):
                xcopy(r).start()
            prologue()
            unsafe = attention()
            if FORCE_FALLBACK:
                unsafe = step == 0
            pl.when(unsafe)(fallback)
            for cp in wcopies():
                cp.wait()

        c0 = pl.multiple_of(step * TD, TD)
        o = ot_s[:, pl.ds(c0, TD)].T.astype(BF)
        x = x_ref[pl.ds(c0, TD), :].astype(F32)
        h1 = x + jnp.dot(o, wo_ref[...], preferred_element_type=F32)
        hn = _ln(h1).astype(BF)
        y = h1
        for f in range(F // FC):
            gt = jnp.dot(hn, wg_ref[:, f * FC:(f + 1) * FC], preferred_element_type=F32)
            up = jnp.dot(hn, wu_ref[:, f * FC:(f + 1) * FC], preferred_element_type=F32)
            a = (gt * jax.nn.sigmoid(gt) * up).astype(BF)
            y = y + jnp.dot(a, wd_ref[f * FC:(f + 1) * FC, :], preferred_element_type=F32)
        o_ref[...] = y.astype(o_ref.dtype)

    def fn(A_x, A_wqkv, A_wo, B_x, B_w_gate, B_w_up, B_w_down):
        x = A_x.reshape(S, D)
        hbm = pl.BlockSpec(memory_space=pl.ANY)
        out = pl.pallas_call(
            kernel,
            grid=(NQ,),
            in_specs=[hbm] * 6,
            out_specs=pl.BlockSpec((TD, D), lambda i: (i, 0)),
            out_shape=jax.ShapeDtypeStruct((S, D), BF),
            scratch_shapes=[
                pltpu.VMEM((S, D), BF), pltpu.VMEM((D, 3 * D), BF),
                pltpu.SemaphoreType.DMA((S // RC + 1,)),
                pltpu.VMEM((D, D), BF), pltpu.VMEM((D, F), BF), pltpu.VMEM((D, F), BF), pltpu.VMEM((F, D), BF),
                pltpu.SemaphoreType.DMA((4,)),
                pltpu.VMEM((D // 2, D), U32), pltpu.VMEM((D, D), U32),
                pltpu.VMEM((NM, S // 2, 128), U32),
                pltpu.VMEM((NM * 16, S), U32),
                pltpu.VMEM((NM * 8, S), U32),
                pltpu.VMEM((NV * 16, S), U32),
                pltpu.VMEM((S, 128), F32),
                pltpu.VMEM((NV * 16, 8, S), F32),
                pltpu.VMEM((64, S), U32),
                pltpu.VMEM((H, S), F32),
                pltpu.VMEM((H, 128), F32),
                pltpu.VMEM((D, S), F32)]
                + [pltpu.VMEM((51, 128, 128), F32)] * 2
                + [pltpu.VMEM((192, S), U32)] * 2
                + [pltpu.SMEM((NZ + 6 * BPU,), I32), pltpu.VMEM((8, TQ), F32), pltpu.VMEM((8, TQ), F32)]
                + [pltpu.VMEM((S // 2 // PSPLIT, TQ), U32)] * (2 * PSPLIT),
            compiler_params=pltpu.CompilerParams(
                dimension_semantics=("arbitrary",), vmem_limit_bytes=110 * 1024 * 1024),
        )(x, A_wqkv, A_wo, B_w_gate, B_w_up, B_w_down)
        return out.reshape(1, S, D)

    return fn


_impl = make_kernel()


@jax.jit
def pallas_sequential_preLN__softmax_full_mha__swiglu_ffn__prompt_kernel(
    A_x: jax.Array,
    A_wqkv: jax.Array,
    A_wo: jax.Array,
    B_x: jax.Array,
    B_w_gate: jax.Array,
    B_w_up: jax.Array,
    B_w_down: jax.Array,
):
    return _impl(A_x, A_wqkv, A_wo, B_x, B_w_gate, B_w_up, B_w_down)
```

```python
import functools
import math

import jax
import jax.numpy as jnp
from jax import lax
import jax.experimental.pallas as pl
import jax.experimental.pallas.tpu as pltpu

S, D, H, DH, F = 2048, 512, 32, 16, 1792
NV = 5
NM = H - NV
CM = NM * DH
TQ = 512
KC = 128
NKC = S // KC
EPS = 1e-5
QSCALE = (DH ** -0.5) * math.log2(math.e)
L_MIN = 2.0 ** -40
L_MAX = 2.0 ** 40
BF = jnp.bfloat16
F32 = jnp.float32
U32 = jnp.uint32
I32 = jnp.int32
ONES = 0x3F803F80
NT = (((1,), (1,)), ((), ()))


def _pack(x):
    return pltpu.bitcast(x, U32)


def _unpack(x):
    return pltpu.bitcast(x, BF)


def _ln(x):
    m = jnp.mean(x, axis=-1, keepdims=True)
    xc = x - m
    v = jnp.mean(xc * xc, axis=-1, keepdims=True)
    return xc * lax.rsqrt(v + EPS)


def _iota(shape, dim):
    return lax.broadcasted_iota(I32, shape, dim)


def make_kernel(RC=512, FC=256, G=2, J=2, LAG=3, PSPLIT=4, HEAD=4, GEND=2, ANCH=2, LSP=8,
                TD=512, DSP=4, PVLAG=0, PRE=1, LOOPM=1, RED=(0, 17, 32, 48), EXT=(), TREE=0, BORD=0, PVS=(15, 16, 16, 16, 31, 32, 32, 47, 48, 48, 48, 63), FORCE_FALLBACK=False):
    NQ = S // TD
    BPU = (128 // (8 * G)) * (S // (128 * J))
    NJ = S // (128 * J)
    Z_K = 3 * BPU
    Z_P = Z_K + 4
    Z_G = Z_P + 4
    Z_T = Z_G + 51
    NZ = Z_T
    CPS = NKC // PSPLIT

    def kernel(x_hbm, wqkv_hbm, wo_hbm, wg_hbm, wu_hbm, wd_hbm, o_ref,
               x_ref, wqkv_ref, xsem, wo_ref, wg_ref, wu_ref, wd_ref, wsem,
               wn_s, wt_s, kr_s, qt_s, vt_s, vtv_s, qn_s, qm_s, ktr_s, ktv_s, nq_s, kmx_s, ot_s,
               q0, q1, p0, p1, z_s, l_s, mm_s, *pab):
        step = pl.program_id(0)
        Q = (q0, q1)
        P = (p0, p1)
        PA = pab[:PSPLIT]
        PB = pab[PSPLIT:]

        def wcopies():
            return [pltpu.make_async_copy(src, dst, wsem.at[n]) for n, (src, dst) in enumerate(
                ((wo_hbm, wo_ref), (wg_hbm, wg_ref), (wu_hbm, wu_ref), (wd_hbm, wd_ref)))]

        def xcopy(r):
            return pltpu.make_async_copy(x_hbm.at[pl.ds(r * RC, RC)], x_ref.at[pl.ds(r * RC, RC)], xsem.at[r])

        def wqkv_copy():
            return pltpu.make_async_copy(wqkv_hbm, wqkv_ref, xsem.at[S // RC])

        def unit_calc(a, i):
            u = jnp.minimum(a * NM + i, 16 * NV - 1)
            return lax.shift_right_logical(u, 4), u & 15

        def gen_qb(jt, dst, a, ds, zi=None):
            j, t = jt
            if zi is not None:
                t = t + z_s[zi]
            for d in ds:
                qn = (qn_s if d < 16 else qm_s)[pl.ds(pl.multiple_of(t * 128, 128), 128), :]
                lane = (48 + 16 * j + d) if d < 16 else j
                v = jnp.take_along_axis(qn, jnp.full((128, 128), lane, I32), axis=1)
                if d == 16:
                    v = v * kmx_s[pl.ds(NM + j, 1), :]
                dst[a * 17 + d] = v
            return v

        def bias_rows(h):
            nq = nq_s[pl.ds(h, 1), :]
            km = jnp.concatenate([kmx_s[pl.ds(h, 1), :]] * (S // 128), axis=1)
            bits = lax.shift_right_logical(pltpu.bitcast((nq * km).astype(BF).astype(F32), U32), jnp.uint32(16))
            row = pl.multiple_of(h * 16 + 8, 8)
            qt_s[pl.ds(row, 8), :] = jnp.where(_iota((8, S), 0) == 0, jnp.broadcast_to(bits, (8, S)), jnp.uint32(0))

        def vpu_mac(par, qsrc, a, b, zi):
            z = z_s[zi]
            zk = z_s[Z_T + par * 3 * BPU + zi]
            g, j = b // NJ, b % NJ
            acc = jnp.concatenate([qsrc[z + (a * 17 + 16), g * 8 * G:(g + 1) * 8 * G, :]] * J, axis=1)
            for d in range(16):
                qb = jnp.concatenate([qsrc[z + (a * 17 + d), g * 8 * G:(g + 1) * 8 * G, :]] * J, axis=1)
                kt = jnp.concatenate([ktr_s[zk + d, :, j * 128 * J:(j + 1) * 128 * J]] * G, axis=0)
                if TREE and d % 2 == 1:
                    acc2 = qb * kt if d == 1 else acc2 + qb * kt
                else:
                    acc = acc + qb * kt
            return acc + acc2 if TREE else acc

        def vpu_exp(pdst, a, b, acc):
            g, j = b // NJ, b % NJ
            pdst[a * 64 + g * 4 * G:a * 64 + (g + 1) * 4 * G, j * 128 * J:(j + 1) * 128 * J] = _pack(
                jnp.exp2(acc).astype(BF))

        def vpu_pv_part(jt, psrc, a, c, acc):
            vt = _unpack(vtv_s[pl.ds(pl.multiple_of(jt[0] * 16, 16), 16), c * 128:(c + 1) * 128])
            pp = _unpack(psrc[a * 64:(a + 1) * 64, c * 128:(c + 1) * 128])
            r = lax.dot_general(vt, pp, NT, preferred_element_type=F32)
            return r if acc is None else acc + r

        def vpu_pv_fin(jt, acc, lmn, lmx):
            j, t = jt
            l = acc[16:17, :]
            ot_s[pl.ds(pl.multiple_of((NM + j) * 16, 16), 16),
                 pl.ds(pl.multiple_of(t * 128, 128), 128)] = acc[:16] / l
            return jnp.minimum(lmn, l), jnp.maximum(lmx, l)

        def scalars(i):
            im1 = jnp.maximum(i - 1, 0)
            return (im1, [unit_calc(a, im1) for a in range(3)], [unit_calc(a, i + 1) for a in range(3)],
                    jnp.minimum(i + 1, NM - 1))

        def half(i, par, pre_sc=None):
            lmn, lmx = mm_s[0:1, :], mm_s[1:2, :]
            lmn2, lmx2 = mm_s[2:3, 0:128], mm_s[3:4, 0:128]
            blocks = [(a, b) for a in range(3) for b in range(BPU)]
            if BORD == 1:
                blocks = [(a, b) for b in range(BPU) for a in range(3)]
            elif BORD == 2:
                blocks = [(a, (b % 8) * NJ + b // 8) for a in range(3) for b in range(BPU)]
            gens = [(a, d) for a in range(3) for d in range(17)]
            nslots = 4 * NKC
            pv_at = {}
            for n in range(12):
                pv_at.setdefault(PVS[n], []).append((n // 4, n % 4))
            if pre_sc is None:
                pre_sc = scalars(i)
            im1, jts_prev, jts_next, hnext = pre_sc
            pending, gvals = [], []
            nb_done = ng_done = npv_done = 0
            vaccs = [None] * 3
            accs = [None] * 4
            ls = [l_s[...]] + [jnp.zeros((8, TQ), F32) for _ in range(4)]
            def scores(slot):
                r, c = slot // NKC, slot % NKC
                if c == 0:
                    qh = qt_s[pl.ds(pl.multiple_of(i * 16, 16), 16), r * TQ:(r + 1) * TQ]
                    wz[0] = _unpack(jnp.concatenate([qh, jnp.zeros((48, TQ), U32)], axis=0))
                    wz[1] = z_s[Z_K + r]
                kc = _unpack(kr_s[i + wz[1], c * KC // 2:(c + 1) * KC // 2, :])
                return jnp.dot(kc, wz[0], preferred_element_type=F32)

            wz = [None, None]
            pre = [scores(n) for n in range(PRE)]
            for _ in range(HEAD):
                a, b = blocks[nb_done]
                vpu_exp(P[par], a, b, vpu_mac(par, Q[par], a, b, nb_done))
                nb_done += 1
            for slot in range(nslots):
                r, c = slot // NKC, slot % NKC
                if RED is None:
                    want = HEAD + ((len(blocks) - HEAD) * (slot + 1)) // nslots
                else:
                    assert len(RED) == HEAD + len(EXT)
                    want = HEAD + 3 * (slot + 1) - sum(1 for x in RED if x <= slot) + sum(1 for x in EXT if x <= slot)
                while nb_done < want:
                    a, b = blocks[nb_done]
                    pending.append((a, b, vpu_mac(par, Q[par], a, b, nb_done)))
                    nb_done += 1
                p = jnp.exp2(pre[slot] if slot < PRE else scores(slot))
                ls[r + 1] = ls[r + 1] + jnp.sum(p.reshape(KC // 8, 8, TQ), axis=0)
                co = (c % CPS) * KC // 2
                (PA if r % 2 == 0 else PB)[c // CPS][co:co + KC // 2, :] = _pack(p.astype(BF))
                while npv_done < nslots and (npv_done + PVLAG <= slot or slot == nslots - 1):
                    r2, c2 = npv_done // NKC, npv_done % NKC
                    hp = im1 if r2 == 0 else i
                    zp = pl.multiple_of(z_s[Z_P + r2] * 8, 8)
                    co2 = (c2 % CPS) * KC // 2
                    vt = _unpack(vt_s[pl.ds(pl.multiple_of(hp * 8, 8), 8), c2 * KC:(c2 + 1) * KC])
                    pr = jnp.dot(vt, _unpack((PB if r2 % 2 == 0 else PA)[c2 // CPS][pl.ds(zp + co2, KC // 2), :]),
                                 preferred_element_type=F32)
                    accs[r2] = pr if c2 == 0 else accs[r2] + pr
                    if c2 == NKC - 1:
                        lt = jnp.sum(ls[r2], axis=0, keepdims=True)
                        lmn, lmx = jnp.minimum(lmn, lt), jnp.maximum(lmx, lt)
                        rp = (r2 - 1) % 4
                        ot_s[pl.ds(pl.multiple_of(hp * 16, 16), DH), rp * TQ:(rp + 1) * TQ] = accs[r2] / lt
                    npv_done += 1
                for a, q in pv_at.get(slot, ()):
                    jt = jts_prev[a]
                    for cc in range(4 * q, 4 * q + 4):
                        vaccs[a] = vpu_pv_part(jt, P[1 - par], a, cc, vaccs[a])
                    if q == 3:
                        lmn2, lmx2 = vpu_pv_fin(jt, vaccs[a], lmn2, lmx2)
                wantg = min(len(gens), (len(gens) * (slot + 1)) // (nslots - GEND) + 1)
                while ng_done < wantg:
                    a, d = gens[ng_done]
                    gv = gen_qb(jts_next[a], Q[1 - par], a, [d], Z_G + ng_done)
                    gvals.append(gv[120:128, :])
                    ng_done += 1
                while len(gvals) > ANCH:
                    one = jnp.exp2(gvals.pop(0) * 0.0)
                    ls[r + 1] = jnp.concatenate([ls[r + 1][:, :128] * one, ls[r + 1][:, 128:]], axis=1)
                while len(pending) > (LAG if slot < nslots - 1 else 0):
                    a, b, ac = pending.pop(0)
                    vpu_exp(P[par], a, b, ac)
            bias_rows(hnext)
            set_ktab(i + 1, 1 - par)
            l_s[...] = ls[4]
            mm_s[0:1, :] = lmn
            mm_s[1:2, :] = lmx
            mm_s[2:3, 0:128] = lmn2
            mm_s[3:4, 0:128] = lmx2

        def set_ktab(i, par):
            for a in range(3):
                v = unit_calc(a, i)[0] * 16
                for b in range(BPU):
                    z_s[Z_T + (par * 3 + a) * BPU + b] = v

        def prologue():
            for b in range(NZ):
                z_s[b] = 0

            def ln1(r, n=0, parts=1):
                pr = RC // parts
                rows = pl.ds(pl.multiple_of(r * RC + n * pr, pr), pr)
                return _pack(_ln(x_ref[rows, :].astype(F32)).astype(BF))

            set_ktab(jnp.int32(0), 0)
            wqkv_copy().wait()
            col = _iota((D, D), 1)
            wq = wqkv_ref[:, 0:D]
            wk = wqkv_ref[:, D:2 * D]
            wn_s[...] = _pack(jnp.where(col < CM, wk, wq))
            wt_s[0:D // 2, :] = _pack(jnp.where(col < CM, wq, wk).T)
            wt_s[D // 2:D, :] = _pack(wqkv_ref[:, 2 * D:3 * D].T)

            def chunk(r, kmax):
                xcopy(r).wait()
                e = jnp.where(_iota((H, D), 1) // DH == _iota((H, D), 0), 1.0, 0.0).astype(BF)
                e2r = _iota((128, 128), 0)
                e2 = jnp.where((e2r >= 48) & ((e2r - 48) // DH == _iota((128, 128), 1)), 1.0, 0.0).astype(BF)
                lane_k = _iota((RC // 2, 128), 1)
                kfill = jnp.where(lane_k == DH, ONES, 0).astype(U32)
                rscale = jnp.where(_iota((D, RC), 0) < CM, QSCALE, 1.0).astype(F32)
                onesblk = jnp.where(_iota((8, RC), 0) == 0, 0x00003F80, 0).astype(U32)
                rows = pl.ds(pl.multiple_of(r * RC, RC), RC)
                prow = pl.ds(pl.multiple_of(r * (RC // 2), RC // 2), RC // 2)
                xs, ks = [], []
                for n in range(LSP):
                    xs.append(_unpack(ln1(r, n, LSP)))
                    ks.append(jnp.dot(xs[-1], _unpack(wn_s[...]), preferred_element_type=F32))
                xn = jnp.concatenate(xs, axis=0)
                kn = jnp.concatenate(ks, axis=0)
                kb = kn.astype(BF)
                kp = _pack(kb)
                for h in range(NM):
                    g, hh = h // 8, h % 8
                    kg = kp[:, g * 128:(g + 1) * 128]
                    if hh:
                        kg = pltpu.roll(kg, 128 - DH * hh, 1)
                    kr_s[h, prow, :] = jnp.where(lane_k < DH, kg, kfill)
                qv = kn[:, 384:512] * QSCALE
                qn_s[rows, :] = qv
                t = lax.dot_general(_unpack(wt_s[...]), xn, NT, preferred_element_type=F32)
                tqk = t[:D] * rscale
                tb = tqk.astype(BF)
                tp = _pack(tb)
                for h in range(NM):
                    qt_s[h * 16:h * 16 + 8, rows] = tp[h * 8:(h + 1) * 8]
                ktv_s[24:64, rows] = tp[CM // 2:]
                for rr in range(NV * DH):
                    ktr_s[rr, :, rows] = jnp.broadcast_to(tqk[CM + rr:CM + rr + 1, :], (8, RC))
                kf = kb.astype(F32)
                kn2 = lax.dot_general(e, (kf * kf).astype(BF), NT, preferred_element_type=F32)
                qv2 = jnp.dot((qv * qv).astype(BF), e2, preferred_element_type=F32)
                qm_s[rows, :] = jnp.sqrt(qv2)
                tf = tb.astype(F32)
                n2 = jnp.dot(e, (tf * tf).astype(BF), preferred_element_type=F32)
                nq_s[:, rows] = jnp.sqrt(n2)
                kmax = jnp.maximum(kmax, jnp.where(_iota((H, RC), 0) < NM, kn2, n2))
                vp = _pack(t[D:].astype(BF))
                vt_s[:, rows] = vp[:CM // 2]
                for j in range(NV):
                    vtv_s[j * 16:j * 16 + 8, rows] = vp[CM // 2 + j * 8:CM // 2 + (j + 1) * 8]
                    vtv_s[j * 16 + 8:j * 16 + 16, rows] = onesblk
                pr = pl.ds(pl.multiple_of(r * (RC // 2 // PSPLIT), 8), RC // 2 // PSPLIT)
                for pp in PB:
                    pp[pr, :] = jnp.full((RC // 2 // PSPLIT, TQ), ONES, U32)
                p1[:, rows] = jnp.full((192, RC), ONES, U32)
                ktv_s[0:24, rows] = jnp.zeros((24, RC), U32)
                for a in ([(2 * r) % 3] if RC == 512 else [r, 2 - 2 * r]):
                    gen_qb(unit_calc(a, 0), q0, a, list(range(16)))
                return kmax

            kmax = lax.fori_loop(0, S // RC, chunk, jnp.zeros((H, RC), F32))
            for cp in wcopies():
                cp.start()
            kmx_s[...] = jnp.broadcast_to(-jnp.sqrt(jnp.max(kmax, axis=1, keepdims=True)), (H, 128))
            bias_rows(0)
            l_s[...] = jnp.ones(l_s.shape, F32)
            mm_s[...] = jnp.ones(mm_s.shape, F32)
            for a in range(3):
                gen_qb(unit_calc(a, jnp.int32(0)), q0, a, [16])

        def attention():
            def body(ii, carry):
                if LOOPM == 0:
                    i = 2 * ii
                    half(i, 0)

                    @pl.when(i + 1 < NM)
                    def _():
                        half(i + 1, 1)
                elif LOOPM == 1:
                    i = 2 * ii

                    @pl.when(i < NM)
                    def _():
                        half(i, 0)

                    @pl.when(i + 1 < NM)
                    def _():
                        half(i + 1, 1)
                elif LOOPM == 3:
                    i = 2 * ii
                    sc = scalars(i)

                    @pl.when(i < NM)
                    def _():
                        half(i, 0, sc)

                    i1 = i + 1
                    sc1 = scalars(i1)

                    @pl.when(i1 < NM)
                    def _():
                        half(i1, 1, sc1)
                else:
                    @pl.when((ii & 1) == 0)
                    def _():
                        half(ii, 0)

                    @pl.when((ii & 1) == 1)
                    def _():
                        half(ii, 1)
                return carry

            lax.fori_loop(0, (NM + 1) // 2 if LOOPM != 2 else NM, body, 0)
            lmn, lmx = mm_s[0:1, :], mm_s[1:2, :]
            lmn2, lmx2 = mm_s[2:3, 0:128], mm_s[3:4, 0:128]
            hp = NM - 1
            pw = jnp.concatenate([pp[...] for pp in PB], axis=0)
            acc = jnp.dot(_unpack(vt_s[hp * 8:(hp + 1) * 8, :]), _unpack(pw), preferred_element_type=F32)
            lt = jnp.sum(l_s[...], axis=0, keepdims=True)
            lmn, lmx = jnp.minimum(lmn, lt), jnp.maximum(lmx, lt)
            ot_s[hp * 16:(hp + 1) * 16, 3 * TQ:] = acc / lt
            for a in range(3):
                if a * NM + NM - 1 >= 16 * NV:
                    continue
                vacc = None
                jt = unit_calc(a, jnp.int32(NM - 1))
                for cc in range(16):
                    vacc = vpu_pv_part(jt, P[(NM - 1) % 2], a, cc, vacc)
                lmn2, lmx2 = vpu_pv_fin(jt, vacc, lmn2, lmx2)
            lo = jnp.minimum(jnp.min(lmn), jnp.min(lmn2))
            hi = jnp.maximum(jnp.max(lmx), jnp.max(lmx2))
            return jnp.logical_not(jnp.logical_and(lo >= L_MIN, hi <= L_MAX))

        def fallback():
            def mxu_item(n, carry):
                h = lax.shift_right_logical(n, 3)
                c0 = pl.multiple_of((n & 7) * 256, 256)
                qh = qt_s[pl.ds(pl.multiple_of(h * 16, 16), 8), pl.ds(c0, 256)]
                w = _unpack(jnp.concatenate([qh, jnp.zeros((56, 256), U32)], axis=0))

                def scores(c):
                    kc = _unpack(kr_s[h, pl.ds(pl.multiple_of(c * 64, 64), 64), :])
                    return jnp.dot(kc, w, preferred_element_type=F32)

                m = lax.fori_loop(
                    0, S // 128,
                    lambda c, m: jnp.maximum(m, jnp.max(scores(c), axis=0, keepdims=True)),
                    jnp.full((1, 256), -jnp.inf, F32))

                def p2(c, carry):
                    l, acc = carry
                    p = jnp.exp2(scores(c) - m)
                    vt = _unpack(vt_s[pl.ds(pl.multiple_of(h * 8, 8), 8), pl.ds(pl.multiple_of(c * 128, 128), 128)])
                    acc = acc + jnp.dot(vt, p.astype(BF), preferred_element_type=F32)
                    return l + jnp.sum(p, axis=0, keepdims=True), acc

                l, acc = lax.fori_loop(0, S // 128, p2, (jnp.zeros((1, 256), F32), jnp.zeros((DH, 256), F32)))
                ot_s[pl.ds(pl.multiple_of(h * DH, DH), DH), pl.ds(c0, 256)] = acc / l
                return carry

            lax.fori_loop(0, NM * 8, mxu_item, 0)

            def vpu_item(u, carry):
                j = lax.shift_right_logical(u, 4)
                t0 = pl.multiple_of((u & 15) * 128, 128)
                lane = _iota((128, 128), 1)
                lo = 48 + 16 * j
                qm = jnp.where((lane >= lo) & (lane < lo + DH), qn_s[pl.ds(t0, 128), :], 0.0).astype(BF)

                def scores(c):
                    kt = _unpack(ktv_s[:, pl.ds(pl.multiple_of(c * 128, 128), 128)])
                    return jnp.dot(qm, kt, preferred_element_type=F32)

                m = lax.fori_loop(0, S // 128, lambda c, m: jnp.maximum(m, scores(c)),
                                  jnp.full((128, 128), -jnp.inf, F32))
                m = jnp.max(m, axis=1, keepdims=True)

                def p2(c, acc):
                    p = jnp.exp2(scores(c) - m).astype(BF)
                    vt = _unpack(vtv_s[pl.ds(pl.multiple_of(j * 16, 16), 16), pl.ds(pl.multiple_of(c * 128, 128), 128)])
                    return acc + lax.dot_general(vt, p, NT, preferred_element_type=F32)

                acc = lax.fori_loop(0, S // 128, p2, jnp.zeros((32, 128), F32))
                ot_s[pl.ds(pl.multiple_of((NM + j) * 16, 16), 16), pl.ds(t0, 128)] = acc[:16] / acc[16:17]
                return carry

            lax.fori_loop(0, NV * 16, vpu_item, 0)

        @pl.when(step == 0)
        def _():
            wqkv_copy().start()
            for r in range(S // RC):
                xcopy(r).start()
            prologue()
            unsafe = attention()
            if FORCE_FALLBACK:
                unsafe = step == 0
            pl.when(unsafe)(fallback)
            for cp in wcopies():
                cp.wait()

        c0 = pl.multiple_of(step * TD, TD)
        RS = TD // DSP
        h1s = []
        for s in range(DSP):
            cs = pl.multiple_of(c0 + s * RS, RS)
            o = ot_s[:, pl.ds(cs, RS)].T.astype(BF)
            x = x_ref[pl.ds(cs, RS), :].astype(F32)
            h1s.append(x + jnp.dot(o, wo_ref[...], preferred_element_type=F32))
        hns, acts = [], []
        for s in range(DSP):
            hn = _ln(h1s[s]).astype(BF)
            hns.append(hn)
            gt = jnp.dot(hn, wg_ref[:, 0:FC], preferred_element_type=F32)
            up = jnp.dot(hn, wu_ref[:, 0:FC], preferred_element_type=F32)
            acts.append((gt * jax.nn.sigmoid(gt) * up).astype(BF))
        hn = jnp.concatenate(hns, axis=0)
        y = jnp.concatenate(h1s, axis=0)
        y = y + jnp.dot(jnp.concatenate(acts, axis=0), wd_ref[0:FC, :], preferred_element_type=F32)
        for f in range(1, F // FC):
            gt = jnp.dot(hn, wg_ref[:, f * FC:(f + 1) * FC], preferred_element_type=F32)
            up = jnp.dot(hn, wu_ref[:, f * FC:(f + 1) * FC], preferred_element_type=F32)
            a = (gt * jax.nn.sigmoid(gt) * up).astype(BF)
            y = y + jnp.dot(a, wd_ref[f * FC:(f + 1) * FC, :], preferred_element_type=F32)
        o_ref[...] = y.astype(o_ref.dtype)

    def fn(A_x, A_wqkv, A_wo, B_x, B_w_gate, B_w_up, B_w_down):
        x = A_x.reshape(S, D)
        hbm = pl.BlockSpec(memory_space=pl.ANY)
        out = pl.pallas_call(
            kernel,
            grid=(NQ,),
            in_specs=[hbm] * 6,
            out_specs=pl.BlockSpec((TD, D), lambda i: (i, 0)),
            out_shape=jax.ShapeDtypeStruct((S, D), BF),
            scratch_shapes=[
                pltpu.VMEM((S, D), BF), pltpu.VMEM((D, 3 * D), BF),
                pltpu.SemaphoreType.DMA((S // RC + 1,)),
                pltpu.VMEM((D, D), BF), pltpu.VMEM((D, F), BF), pltpu.VMEM((D, F), BF), pltpu.VMEM((F, D), BF),
                pltpu.SemaphoreType.DMA((4,)),
                pltpu.VMEM((D // 2, D), U32), pltpu.VMEM((D, D), U32),
                pltpu.VMEM((NM, S // 2, 128), U32),
                pltpu.VMEM((NM * 16, S), U32),
                pltpu.VMEM((NM * 8, S), U32),
                pltpu.VMEM((NV * 16, S), U32),
                pltpu.VMEM((S, 128), F32),
                pltpu.VMEM((S, 128), F32),
                pltpu.VMEM((NV * 16, 8, S), F32),
                pltpu.VMEM((64, S), U32),
                pltpu.VMEM((H, S), F32),
                pltpu.VMEM((H, 128), F32),
                pltpu.VMEM((D, S), F32)]
                + [pltpu.VMEM((51, 128, 128), F32)] * 2
                + [pltpu.VMEM((192, S), U32)] * 2
                + [pltpu.SMEM((NZ + 6 * BPU,), I32), pltpu.VMEM((8, TQ), F32), pltpu.VMEM((8, TQ), F32)]
                + [pltpu.VMEM((S // 2 // PSPLIT, TQ), U32)] * (2 * PSPLIT),
            compiler_params=pltpu.CompilerParams(
                dimension_semantics=("arbitrary",), vmem_limit_bytes=110 * 1024 * 1024),
        )(x, A_wqkv, A_wo, B_w_gate, B_w_up, B_w_down)
        return out.reshape(1, S, D)

    return fn


_impl = make_kernel()


@jax.jit
def pallas_sequential_preLN__softmax_full_mha__swiglu_ffn__prompt_kernel(
    A_x: jax.Array,
    A_wqkv: jax.Array,
    A_wo: jax.Array,
    B_x: jax.Array,
    B_w_gate: jax.Array,
    B_w_up: jax.Array,
    B_w_down: jax.Array,
):
    return _impl(A_x, A_wqkv, A_wo, B_x, B_w_gate, B_w_up, B_w_down)
```

```python
import math

import jax
import jax.numpy as jnp
from jax import lax
import jax.experimental.pallas as pl
import jax.experimental.pallas.tpu as pltpu

S, D, H, DH, F = 2048, 512, 32, 16, 1792
NV = 5
NM = H - NV
CM = NM * DH
TQ = 512
KC = 128
NKC = S // KC
RC = 512
LSP = 8
TD = 512
DSP = 4
FC = 256
PSPLIT = 4
CPS = NKC // PSPLIT
BPU = 64
NJ = 8
LAG = 3
GEND = 2
ANCH = 2
RED = (0, 17, 32, 48)
PVS = (15, 16, 16, 16, 31, 32, 32, 47, 48, 48, 48, 63)
HEAD = len(RED)
Z_K = 3 * BPU
Z_P = Z_K + 4
Z_G = Z_P + 4
Z_T = Z_G + 51
EPS = 1e-5
QSCALE = (DH ** -0.5) * math.log2(math.e)
L_MIN = 2.0 ** -40
L_MAX = 2.0 ** 24
BF = jnp.bfloat16
F32 = jnp.float32
U32 = jnp.uint32
I32 = jnp.int32
ONES = 0x3F803F80
NT = (((1,), (1,)), ((), ()))


def _pack(x):
    return pltpu.bitcast(x, U32)


def _unpack(x):
    return pltpu.bitcast(x, BF)


def _ln(x):
    m = jnp.mean(x, axis=-1, keepdims=True)
    xc = x - m
    v = jnp.mean(xc * xc, axis=-1, keepdims=True)
    return xc * lax.rsqrt(v + EPS)


def _iota(shape, dim):
    return lax.broadcasted_iota(I32, shape, dim)


def make_kernel(FORCE_FALLBACK=False):
    def kernel(x_hbm, wqkv_hbm, wo_hbm, wg_hbm, wu_hbm, wd_hbm, o_ref,
               x_ref, wqkv_ref, xsem, wo_ref, wg_ref, wu_ref, wd_ref, wsem,
               wn_s, wt_s, kr_s, qt_s, vt_s, vtv_s, qn_s, qm_s, ktr_s, ktv_s, nq_s, kmx_s, ot_s,
               q0, q1, p0, p1, z_s, l_s, mm_s, *pab):
        step = pl.program_id(0)
        Q = (q0, q1)
        P = (p0, p1)
        PA = pab[:PSPLIT]
        PB = pab[PSPLIT:]

        def wcopies():
            return [pltpu.make_async_copy(src, dst, wsem.at[n]) for n, (src, dst) in enumerate(
                ((wo_hbm, wo_ref), (wg_hbm, wg_ref), (wu_hbm, wu_ref), (wd_hbm, wd_ref)))]

        def xcopy(r):
            return pltpu.make_async_copy(x_hbm.at[pl.ds(r * RC, RC)], x_ref.at[pl.ds(r * RC, RC)], xsem.at[r])

        def wqkv_copy():
            return pltpu.make_async_copy(wqkv_hbm, wqkv_ref, xsem.at[S // RC])

        def unit_calc(a, i):
            u = jnp.minimum(a * NM + i, 16 * NV - 1)
            return lax.shift_right_logical(u, 4), u & 15

        def gen_qb(jt, dst, a, ds, zi=None):
            j, t = jt
            if zi is not None:
                t = t + z_s[zi]
            for d in ds:
                qn = (qn_s if d < 16 else qm_s)[pl.ds(pl.multiple_of(t * 128, 128), 128), :]
                lane = (48 + 16 * j + d) if d < 16 else j
                v = jnp.take_along_axis(qn, jnp.full((128, 128), lane, I32), axis=1)
                if d == 16:
                    v = v * kmx_s[pl.ds(NM + j, 1), :]
                dst[a * 17 + d] = v
            return v

        def bias_rows(h):
            nq = nq_s[pl.ds(h, 1), :]
            km = jnp.concatenate([kmx_s[pl.ds(h, 1), :]] * (S // 128), axis=1)
            bits = lax.shift_right_logical(pltpu.bitcast((nq * km).astype(BF).astype(F32), U32), jnp.uint32(16))
            row = pl.multiple_of(h * 16 + 8, 8)
            qt_s[pl.ds(row, 8), :] = jnp.where(_iota((8, S), 0) == 0, jnp.broadcast_to(bits, (8, S)), jnp.uint32(0))

        def vpu_mac(par, a, b, zi):
            z = z_s[zi]
            zk = z_s[Z_T + par * 3 * BPU + zi]
            g, j = b // NJ, b % NJ
            acc = jnp.concatenate([Q[par][z + (a * 17 + 16), g * 16:(g + 1) * 16, :]] * 2, axis=1)
            for d in range(DH):
                qb = jnp.concatenate([Q[par][z + (a * 17 + d), g * 16:(g + 1) * 16, :]] * 2, axis=1)
                kt = jnp.concatenate([ktr_s[zk + d, :, j * 256:(j + 1) * 256]] * 2, axis=0)
                acc = acc + qb * kt
            return acc

        def vpu_exp(par, a, b, acc):
            g, j = b // NJ, b % NJ
            P[par][a * 64 + g * 8:a * 64 + (g + 1) * 8, j * 256:(j + 1) * 256] = _pack(jnp.exp2(acc).astype(BF))

        def vpu_pv_part(jt, psrc, a, c, acc):
            vt = _unpack(vtv_s[pl.ds(pl.multiple_of(jt[0] * 16, 16), 16), c * 128:(c + 1) * 128])
            pp = _unpack(psrc[a * 64:(a + 1) * 64, c * 128:(c + 1) * 128])
            r = lax.dot_general(vt, pp, NT, preferred_element_type=F32)
            return r if acc is None else acc + r

        def vpu_pv_fin(jt, acc, lmn, lmx):
            j, t = jt
            l = acc[16:17, :]
            ot_s[pl.ds(pl.multiple_of((NM + j) * 16, 16), 16),
                 pl.ds(pl.multiple_of(t * 128, 128), 128)] = acc[:16] / l
            return jnp.minimum(lmn, l), jnp.maximum(lmx, l)

        def set_ktab(i, par):
            for a in range(3):
                v = unit_calc(a, i)[0] * 16
                for b in range(BPU):
                    z_s[Z_T + (par * 3 + a) * BPU + b] = v

        def half(i, par):
            lmn, lmx = mm_s[0:1, :], mm_s[1:2, :]
            lmn2, lmx2 = mm_s[2:3, 0:128], mm_s[3:4, 0:128]
            blocks = [(a, b) for a in range(3) for b in range(BPU)]
            gens = [(a, d) for a in range(3) for d in range(17)]
            nslots = 4 * NKC
            im1 = jnp.maximum(i - 1, 0)
            jts_prev = [unit_calc(a, im1) for a in range(3)]
            jts_next = [unit_calc(a, i + 1) for a in range(3)]
            hnext = jnp.minimum(i + 1, NM - 1)
            pending, gvals = [], []
            nb_done = ng_done = 0
            vaccs = [None] * 3
            acc = None
            ls = [l_s[...]] + [jnp.zeros((8, TQ), F32) for _ in range(4)]
            wz = [None, None]

            def scores(slot):
                r, c = slot // NKC, slot % NKC
                if c == 0:
                    qh = qt_s[pl.ds(pl.multiple_of(i * 16, 16), 16), r * TQ:(r + 1) * TQ]
                    wz[0] = _unpack(jnp.concatenate([qh, jnp.zeros((48, TQ), U32)], axis=0))
                    wz[1] = z_s[Z_K + r]
                kc = _unpack(kr_s[i + wz[1], c * KC // 2:(c + 1) * KC // 2, :])
                return jnp.dot(kc, wz[0], preferred_element_type=F32)

            s0 = scores(0)
            for _ in range(HEAD):
                a, b = blocks[nb_done]
                vpu_exp(par, a, b, vpu_mac(par, a, b, nb_done))
                nb_done += 1
            for slot in range(nslots):
                r, c = slot // NKC, slot % NKC
                want = HEAD + 3 * (slot + 1) - sum(1 for x in RED if x <= slot)
                while nb_done < want:
                    a, b = blocks[nb_done]
                    pending.append((a, b, vpu_mac(par, a, b, nb_done)))
                    nb_done += 1
                p = jnp.exp2(s0 if slot == 0 else scores(slot))
                ls[r + 1] = ls[r + 1] + jnp.sum(p.reshape(KC // 8, 8, TQ), axis=0)
                co = (c % CPS) * KC // 2
                (PA if r % 2 == 0 else PB)[c // CPS][co:co + KC // 2, :] = _pack(p.astype(BF))
                hp = im1 if r == 0 else i
                zp = pl.multiple_of(z_s[Z_P + r] * 8, 8)
                vt = _unpack(vt_s[pl.ds(pl.multiple_of(hp * 8, 8), 8), c * KC:(c + 1) * KC])
                pr = jnp.dot(vt, _unpack((PB if r % 2 == 0 else PA)[c // CPS][pl.ds(zp + co, KC // 2), :]),
                             preferred_element_type=F32)
                acc = pr if c == 0 else acc + pr
                if c == NKC - 1:
                    lt = jnp.sum(ls[r], axis=0, keepdims=True)
                    lmn, lmx = jnp.minimum(lmn, lt), jnp.maximum(lmx, lt)
                    rp = (r - 1) % 4
                    ot_s[pl.ds(pl.multiple_of(hp * 16, 16), DH), rp * TQ:(rp + 1) * TQ] = acc / lt
                for n in range(12):
                    if PVS[n] == slot:
                        a, q = n // 4, n % 4
                        for cc in range(4 * q, 4 * q + 4):
                            vaccs[a] = vpu_pv_part(jts_prev[a], P[1 - par], a, cc, vaccs[a])
                        if q == 3:
                            lmn2, lmx2 = vpu_pv_fin(jts_prev[a], vaccs[a], lmn2, lmx2)
                wantg = min(len(gens), (len(gens) * (slot + 1)) // (nslots - GEND) + 1)
                while ng_done < wantg:
                    a, d = gens[ng_done]
                    gv = gen_qb(jts_next[a], Q[1 - par], a, [d], Z_G + ng_done)
                    gvals.append(gv[120:128, :])
                    ng_done += 1
                while len(gvals) > ANCH:
                    one = jnp.exp2(gvals.pop(0) * 0.0)
                    ls[r + 1] = jnp.concatenate([ls[r + 1][:, :128] * one, ls[r + 1][:, 128:]], axis=1)
                while len(pending) > (LAG if slot < nslots - 1 else 0):
                    a, b, ac = pending.pop(0)
                    vpu_exp(par, a, b, ac)
            bias_rows(hnext)
            set_ktab(i + 1, 1 - par)
            l_s[...] = ls[4]
            mm_s[0:1, :] = lmn
            mm_s[1:2, :] = lmx
            mm_s[2:3, 0:128] = lmn2
            mm_s[3:4, 0:128] = lmx2

        def prologue():
            for b in range(Z_T):
                z_s[b] = 0
            set_ktab(jnp.int32(0), 0)
            wqkv_copy().wait()
            col = _iota((D, D), 1)
            wq = wqkv_ref[:, 0:D]
            wk = wqkv_ref[:, D:2 * D]
            wn_s[...] = _pack(jnp.where(col < CM, wk, wq))
            wt_s[0:D // 2, :] = _pack(jnp.where(col < CM, wq, wk).T)
            wt_s[D // 2:D, :] = _pack(wqkv_ref[:, 2 * D:3 * D].T)

            def chunk(r, kmax):
                xcopy(r).wait()
                e = jnp.where(_iota((H, D), 1) // DH == _iota((H, D), 0), 1.0, 0.0).astype(BF)
                e2r = _iota((128, 128), 0)
                e2 = jnp.where((e2r >= 48) & ((e2r - 48) // DH == _iota((128, 128), 1)), 1.0, 0.0).astype(BF)
                lane_k = _iota((RC // 2, 128), 1)
                kfill = jnp.where(lane_k == DH, ONES, 0).astype(U32)
                rscale = jnp.where(_iota((D, RC), 0) < CM, QSCALE, 1.0).astype(F32)
                onesblk = jnp.where(_iota((8, RC), 0) == 0, 0x00003F80, 0).astype(U32)
                rows = pl.ds(pl.multiple_of(r * RC, RC), RC)
                prow = pl.ds(pl.multiple_of(r * (RC // 2), RC // 2), RC // 2)
                xs, ks = [], []
                sub = RC // LSP
                for n in range(LSP):
                    xr = pl.ds(pl.multiple_of(r * RC + n * sub, sub), sub)
                    xs.append(_unpack(_pack(_ln(x_ref[xr, :].astype(F32)).astype(BF))))
                    ks.append(jnp.dot(xs[-1], _unpack(wn_s[...]), preferred_element_type=F32))
                xn = jnp.concatenate(xs, axis=0)
                kn = jnp.concatenate(ks, axis=0)
                kb = kn.astype(BF)
                kp = _pack(kb)
                for h in range(NM):
                    g, hh = h // 8, h % 8
                    kg = kp[:, g * 128:(g + 1) * 128]
                    if hh:
                        kg = pltpu.roll(kg, 128 - DH * hh, 1)
                    kr_s[h, prow, :] = jnp.where(lane_k < DH, kg, kfill)
                qv = kn[:, 384:512] * QSCALE
                qn_s[rows, :] = qv
                t = lax.dot_general(_unpack(wt_s[...]), xn, NT, preferred_element_type=F32)
                tqk = t[:D] * rscale
                tb = tqk.astype(BF)
                tp = _pack(tb)
                for h in range(NM):
                    qt_s[h * 16:h * 16 + 8, rows] = tp[h * 8:(h + 1) * 8]
                ktv_s[24:64, rows] = tp[CM // 2:]
                for rr in range(NV * DH):
                    ktr_s[rr, :, rows] = jnp.broadcast_to(tqk[CM + rr:CM + rr + 1, :], (8, RC))
                kf = kb.astype(F32)
                kn2 = lax.dot_general(e, (kf * kf).astype(BF), NT, preferred_element_type=F32)
                qv2 = jnp.dot((qv * qv).astype(BF), e2, preferred_element_type=F32)
                qm_s[rows, :] = jnp.sqrt(qv2)
                tf = tb.astype(F32)
                n2 = jnp.dot(e, (tf * tf).astype(BF), preferred_element_type=F32)
                nq_s[:, rows] = jnp.sqrt(n2)
                kmax = jnp.maximum(kmax, jnp.where(_iota((H, RC), 0) < NM, kn2, n2))
                vp = _pack(t[D:].astype(BF))
                vt_s[:, rows] = vp[:CM // 2]
                for j in range(NV):
                    vtv_s[j * 16:j * 16 + 8, rows] = vp[CM // 2 + j * 8:CM // 2 + (j + 1) * 8]
                    vtv_s[j * 16 + 8:j * 16 + 16, rows] = onesblk
                pr = pl.ds(pl.multiple_of(r * (RC // 2 // PSPLIT), 8), RC // 2 // PSPLIT)
                for pp in PB:
                    pp[pr, :] = jnp.full((RC // 2 // PSPLIT, TQ), ONES, U32)
                p1[:, rows] = jnp.full((192, RC), ONES, U32)
                ktv_s[0:24, rows] = jnp.zeros((24, RC), U32)
                a = (2 * r) % 3
                gen_qb(unit_calc(a, 0), q0, a, list(range(16)))
                return kmax

            kmax = lax.fori_loop(0, S // RC, chunk, jnp.zeros((H, RC), F32))
            for cp in wcopies():
                cp.start()
            kmx_s[...] = jnp.broadcast_to(-jnp.sqrt(jnp.max(kmax, axis=1, keepdims=True)), (H, 128))
            bias_rows(0)
            l_s[...] = jnp.ones(l_s.shape, F32)
            mm_s[...] = jnp.ones(mm_s.shape, F32)
            for a in range(3):
                gen_qb(unit_calc(a, jnp.int32(0)), q0, a, [16])

        def attention():
            def body(ii, carry):
                i = 2 * ii

                @pl.when(i < NM)
                def _():
                    half(i, 0)

                @pl.when(i + 1 < NM)
                def _():
                    half(i + 1, 1)

                return carry

            lax.fori_loop(0, (NM + 1) // 2, body, 0)
            lmn, lmx = mm_s[0:1, :], mm_s[1:2, :]
            lmn2, lmx2 = mm_s[2:3, 0:128], mm_s[3:4, 0:128]
            hp = NM - 1
            pw = jnp.concatenate([pp[...] for pp in PB], axis=0)
            acc = jnp.dot(_unpack(vt_s[hp * 8:(hp + 1) * 8, :]), _unpack(pw), preferred_element_type=F32)
            lt = jnp.sum(l_s[...], axis=0, keepdims=True)
            lmn, lmx = jnp.minimum(lmn, lt), jnp.maximum(lmx, lt)
            ot_s[hp * 16:(hp + 1) * 16, 3 * TQ:] = acc / lt
            for a in range(3):
                if a * NM + NM - 1 >= 16 * NV:
                    continue
                vacc = None
                jt = unit_calc(a, jnp.int32(NM - 1))
                for cc in range(16):
                    vacc = vpu_pv_part(jt, P[(NM - 1) % 2], a, cc, vacc)
                lmn2, lmx2 = vpu_pv_fin(jt, vacc, lmn2, lmx2)
            lo = jnp.minimum(jnp.min(lmn), jnp.min(lmn2))
            hi = jnp.maximum(jnp.max(lmx), jnp.max(lmx2))
            return jnp.logical_not(jnp.logical_and(lo >= L_MIN, hi <= L_MAX))

        def fallback():
            def mxu_item(n, carry):
                h = lax.shift_right_logical(n, 3)
                c0 = pl.multiple_of((n & 7) * 256, 256)
                qh = qt_s[pl.ds(pl.multiple_of(h * 16, 16), 8), pl.ds(c0, 256)]
                w = _unpack(jnp.concatenate([qh, jnp.zeros((56, 256), U32)], axis=0))

                def scores(c):
                    kc = _unpack(kr_s[h, pl.ds(pl.multiple_of(c * 64, 64), 64), :])
                    return jnp.dot(kc, w, preferred_element_type=F32)

                m = lax.fori_loop(
                    0, S // 128,
                    lambda c, m: jnp.maximum(m, jnp.max(scores(c), axis=0, keepdims=True)),
                    jnp.full((1, 256), -jnp.inf, F32))

                def p2(c, carry):
                    l, acc = carry
                    p = jnp.exp2(scores(c) - m)
                    vt = _unpack(vt_s[pl.ds(pl.multiple_of(h * 8, 8), 8), pl.ds(pl.multiple_of(c * 128, 128), 128)])
                    acc = acc + jnp.dot(vt, p.astype(BF), preferred_element_type=F32)
                    return l + jnp.sum(p, axis=0, keepdims=True), acc

                l, acc = lax.fori_loop(0, S // 128, p2, (jnp.zeros((1, 256), F32), jnp.zeros((DH, 256), F32)))
                ot_s[pl.ds(pl.multiple_of(h * DH, DH), DH), pl.ds(c0, 256)] = acc / l
                return carry

            lax.fori_loop(0, NM * 8, mxu_item, 0)

            def vpu_item(u, carry):
                j = lax.shift_right_logical(u, 4)
                t0 = pl.multiple_of((u & 15) * 128, 128)
                lane = _iota((128, 128), 1)
                lo = 48 + 16 * j
                qm = jnp.where((lane >= lo) & (lane < lo + DH), qn_s[pl.ds(t0, 128), :], 0.0).astype(BF)

                def scores(c):
                    kt = _unpack(ktv_s[:, pl.ds(pl.multiple_of(c * 128, 128), 128)])
                    return jnp.dot(qm, kt, preferred_element_type=F32)

                m = lax.fori_loop(0, S // 128, lambda c, m: jnp.maximum(m, scores(c)),
                                  jnp.full((128, 128), -jnp.inf, F32))
                m = jnp.max(m, axis=1, keepdims=True)

                def p2(c, acc):
                    p = jnp.exp2(scores(c) - m).astype(BF)
                    vt = _unpack(vtv_s[pl.ds(pl.multiple_of(j * 16, 16), 16),
                                       pl.ds(pl.multiple_of(c * 128, 128), 128)])
                    return acc + lax.dot_general(vt, p, NT, preferred_element_type=F32)

                acc = lax.fori_loop(0, S // 128, p2, jnp.zeros((32, 128), F32))
                ot_s[pl.ds(pl.multiple_of((NM + j) * 16, 16), 16), pl.ds(t0, 128)] = acc[:16] / acc[16:17]
                return carry

            lax.fori_loop(0, NV * 16, vpu_item, 0)

        @pl.when(step == 0)
        def _():
            wqkv_copy().start()
            for r in range(S // RC):
                xcopy(r).start()
            prologue()
            unsafe = attention()
            if FORCE_FALLBACK:
                unsafe = step == 0
            pl.when(unsafe)(fallback)
            for cp in wcopies():
                cp.wait()

        c0 = pl.multiple_of(step * TD, TD)
        rs = TD // DSP
        h1s = []
        for s in range(DSP):
            cs = pl.multiple_of(c0 + s * rs, rs)
            o = ot_s[:, pl.ds(cs, rs)].T.astype(BF)
            x = x_ref[pl.ds(cs, rs), :].astype(F32)
            h1s.append(x + jnp.dot(o, wo_ref[...], preferred_element_type=F32))
        hns, acts = [], []
        for s in range(DSP):
            hn = _ln(h1s[s]).astype(BF)
            hns.append(hn)
            gt = jnp.dot(hn, wg_ref[:, 0:FC], preferred_element_type=F32)
            up = jnp.dot(hn, wu_ref[:, 0:FC], preferred_element_type=F32)
            acts.append((gt * jax.nn.sigmoid(gt) * up).astype(BF))
        hn = jnp.concatenate(hns, axis=0)
        y = jnp.concatenate(h1s, axis=0)
        y = y + jnp.dot(jnp.concatenate(acts, axis=0), wd_ref[0:FC, :], preferred_element_type=F32)
        for f in range(1, F // FC):
            gt = jnp.dot(hn, wg_ref[:, f * FC:(f + 1) * FC], preferred_element_type=F32)
            up = jnp.dot(hn, wu_ref[:, f * FC:(f + 1) * FC], preferred_element_type=F32)
            a = (gt * jax.nn.sigmoid(gt) * up).astype(BF)
            y = y + jnp.dot(a, wd_ref[f * FC:(f + 1) * FC, :], preferred_element_type=F32)
        o_ref[...] = y.astype(o_ref.dtype)

    def fn(A_x, A_wqkv, A_wo, B_x, B_w_gate, B_w_up, B_w_down):
        x = A_x.reshape(S, D)
        hbm = pl.BlockSpec(memory_space=pl.ANY)
        out = pl.pallas_call(
            kernel,
            grid=(S // TD,),
            in_specs=[hbm] * 6,
            out_specs=pl.BlockSpec((TD, D), lambda i: (i, 0)),
            out_shape=jax.ShapeDtypeStruct((S, D), BF),
            scratch_shapes=[
                pltpu.VMEM((S, D), BF), pltpu.VMEM((D, 3 * D), BF),
                pltpu.SemaphoreType.DMA((S // RC + 1,)),
                pltpu.VMEM((D, D), BF), pltpu.VMEM((D, F), BF), pltpu.VMEM((D, F), BF), pltpu.VMEM((F, D), BF),
                pltpu.SemaphoreType.DMA((4,)),
                pltpu.VMEM((D // 2, D), U32),
                pltpu.VMEM((D, D), U32),
                pltpu.VMEM((NM, S // 2, 128), U32),
                pltpu.VMEM((NM * 16, S), U32),
                pltpu.VMEM((NM * 8, S), U32),
                pltpu.VMEM((NV * 16, S), U32),
                pltpu.VMEM((S, 128), F32),
                pltpu.VMEM((S, 128), F32),
                pltpu.VMEM((NV * 16, 8, S), F32),
                pltpu.VMEM((64, S), U32),
                pltpu.VMEM((H, S), F32),
                pltpu.VMEM((H, 128), F32),
                pltpu.VMEM((D, S), F32)]
                + [pltpu.VMEM((51, 128, 128), F32)] * 2
                + [pltpu.VMEM((192, S), U32)] * 2
                + [pltpu.SMEM((Z_T + 6 * BPU,), I32), pltpu.VMEM((8, TQ), F32), pltpu.VMEM((8, TQ), F32)]
                + [pltpu.VMEM((S // 2 // PSPLIT, TQ), U32)] * (2 * PSPLIT),
            compiler_params=pltpu.CompilerParams(
                dimension_semantics=("arbitrary",), vmem_limit_bytes=110 * 1024 * 1024),
        )(x, A_wqkv, A_wo, B_w_gate, B_w_up, B_w_down)
        return out.reshape(1, S, D)

    return fn


_impl = make_kernel()


@jax.jit
def pallas_sequential_preLN__softmax_full_mha__swiglu_ffn__prompt_kernel(
    A_x: jax.Array,
    A_wqkv: jax.Array,
    A_wo: jax.Array,
    B_x: jax.Array,
    B_w_gate: jax.Array,
    B_w_up: jax.Array,
    B_w_down: jax.Array,
):
    return _impl(A_x, A_wqkv, A_wo, B_x, B_w_gate, B_w_up, B_w_down)
```
